```python
import os as _os
_os.environ.setdefault("JAX_PLATFORMS", "cpu")
import jax
import jax.numpy as jnp

def _softmax(x, axis=-1):
    return jax.nn.softmax(x, axis=axis)
def _gelu(x):
    return jax.nn.gelu(x, approximate=True)
def _silu(x):
    return jax.nn.silu(x)
def _sigmoid(x):
    return jax.nn.sigmoid(x)
def _layernorm(x, axis=-1, eps=1e-5):
    m = jnp.mean(x, axis=axis, keepdims=True)
    v = jnp.var(x, axis=axis, keepdims=True)
    return (x - m) / jnp.sqrt(v + eps)
def _scatter_add(tgt, idx, src, axis=0):
    return tgt.at[idx].add(src)
def _segment_sum(src, seg, n):
    return jax.ops.segment_sum(src, seg, n)
class _Rng:
    def __init__(self, key):
        self._k = key
    def _next(self):
        self._k, sub = jax.random.split(self._k)
        return sub
    def normal(self, shape):
        return jax.random.normal(self._next(), shape, dtype=jnp.bfloat16)
    def randint(self, lo, hi, shape):
        return jax.random.randint(self._next(), shape, lo, hi, dtype=jnp.int32)
    def uniform(self, shape, lo=0.0, hi=1.0):
        return jax.random.uniform(self._next(), shape, jnp.bfloat16, lo, hi)
    def permutation(self, n):
        return jax.random.permutation(self._next(), n)


kernel_name = 'gated_mix__linear_attn_block__swiglu_ffn__prompt'

def setup_inputs():
    _rng = _Rng(jax.random.key(int.from_bytes(__import__("os").urandom(4), "little")))
    _w = (lambda a: (lambda t: t.astype(jnp.bfloat16) if jnp.issubdtype(t.dtype, jnp.floating) else t)(jnp.asarray(a)))
    def _A_setup():
        B, S, D = 1, 2048, 512
        return {
            "x": _w((lambda *s: _rng.normal(s) * 0.05)(B, S, D)),
            "wqkv": _w((lambda *s: _rng.normal(s) * 0.8)(D, 3 * D)),
            "wo": _w((lambda *s: _rng.normal(s) * 0.05)(D, D)),
        }
    _A_in = _A_setup()

    def _B_setup():
        B, S, D, F = 1, 2048, 512, 1792
        return {
            "x": _w((lambda *s: _rng.normal(s) * 0.05)(B, S, D)),
            "w_gate": _w((lambda *s: _rng.normal(s) * 0.1)(D, F)),
            "w_up": _w((lambda *s: _rng.normal(s) * 0.1)(D, F)),
            "w_down": _w((lambda *s: _rng.normal(s) * 0.1)(F, D)),
        }
    _B_in = _B_setup()

    return {
        "A_x": _A_in["x"],
        "A_wqkv": _A_in["wqkv"],
        "A_wo": _A_in["wo"],
        "B_x": _B_in["x"],
        "B_w_gate": _B_in["w_gate"],
        "B_w_up": _B_in["w_up"],
        "B_w_down": _B_in["w_down"],
        "gate_w": _w((lambda *s: _rng.normal(s) * 0.05)(512) * 16.0),
    }

def reference(A_x, A_wqkv, A_wo, B_x, B_w_gate, B_w_up, B_w_down, gate_w):
    def _A_ref(x, wqkv, wo):
        B, S, D = x.shape
        H = 32; Dh = D // H
        qkv = (lambda x, *d: x.transpose(*d))((x @ wqkv).reshape(B, S, 3, H, Dh), 2, 0, 3, 1, 4)
        q, k, v = qkv[0], qkv[1], qkv[2]
        phi = lambda t: jnp.where(t > 0, t + 1, jnp.exp(t)) + 1e-6
        pq, pk = phi(q), phi(k)
        kv = jnp.einsum("bhsd,bhse->bhde", pk, v)
        z = jnp.einsum("bhsd->bhd", pk)
        num = jnp.einsum("bhqd,bhde->bhqe", pq, kv)
        den = jnp.einsum("bhqd,bhd->bhq", pq, z)[..., None] + 1e-6
        o = num / den
        return (lambda x, *d: x.transpose(*d))(o, 0, 2, 1, 3).reshape(B, S, D) @ wo

    def _B_ref(x, w_gate, w_up, w_down):
        g = _silu(x @ w_gate)
        u = x @ w_up
        return (g * u) @ w_down

    x = A_x
    g = _sigmoid((x * gate_w).sum(-1, keepdims=True))
    a = _A_ref(x, A_wqkv, A_wo)
    b = _B_ref(x, B_w_gate, B_w_up, B_w_down)
    return g * a + (1 - g) * b
```

```python
import functools
import jax
import jax.numpy as jnp
from jax import lax
import jax.experimental.pallas as pl
import jax.experimental.pallas.tpu as pltpu

F32 = jnp.float32
BF16 = jnp.bfloat16
U32 = jnp.uint32
NT = (((1,), (1,)), ((), ()))
H = 32


def _phi(t):
    return jnp.where(t > 0, t + 1.0, jnp.exp(t)) + 1e-6


def _sigmoid(t):
    return 0.5 * jnp.tanh(0.5 * t) + 0.5


def make(xsplit=(256, 512, 1280), KT=512, QT=128, T2=512, subs=(256, 256), fcs=(256,) * 7, nosem=True,
         wq_blk=1, kv_at=1, m_at=16, g_early=False):
    assert sum(subs) == T2

    def kernel(x_hbm, wqkv_hbm, wo_hbm, wg_hbm, wu_hbm, wd_hbm, gw_hbm, o_hbm,
               x_v, wq_v, wk_v, wv_v, wo_v, wg_v, wu_v, wd_v, gw_v, wqp_v, t32_v, p_acc, z_acc, zt_v,
               kv_v, m_v, r_v, g_v, o_v, sem, osem):
        S, D = x_v.shape
        F = wg_v.shape[1]
        Dh = D // H
        NB = D // 128
        NP = Dh // 2
        n2 = S // T2
        nx = len(xsplit)
        xoff = [sum(xsplit[:i]) for i in range(nx)]

        xcp = [pltpu.make_async_copy(x_hbm.at[pl.ds(xoff[i], xsplit[i])], x_v.at[pl.ds(xoff[i], xsplit[i])], sem.at[i])
               for i in range(nx)]
        cp_wk = pltpu.make_async_copy(wqkv_hbm.at[:, pl.ds(D, D)], wk_v, sem.at[nx + 0])
        cp_wq = pltpu.make_async_copy(wqkv_hbm.at[:, pl.ds(0, D)], wq_v, sem.at[nx + 1])
        cp_wv = pltpu.make_async_copy(wqkv_hbm.at[:, pl.ds(2 * D, D)], wv_v, sem.at[nx + 2])
        cp_wo = pltpu.make_async_copy(wo_hbm, wo_v, sem.at[nx + 3])
        cp_wg = pltpu.make_async_copy(wg_hbm, wg_v, sem.at[nx + 4])
        cp_wu = pltpu.make_async_copy(wu_hbm, wu_v, sem.at[nx + 5])
        cp_wd = pltpu.make_async_copy(wd_hbm, wd_v, sem.at[nx + 6])
        cp_gw = pltpu.make_async_copy(gw_hbm, gw_v, sem.at[nx + 7])

        xcp[0].start()
        cp_wk.start()
        cp_gw.start()
        for i in range(1, nx):
            if i == wq_blk:
                cp_wq.start()
            xcp[i].start()
        cp_wv.start()
        cp_wo.start()
        cp_wg.start()
        cp_wu.start()
        cp_wd.start()

        def g_tile(r0, rows):
            gw = gw_v[...].astype(F32).reshape(1, D)
            xt = x_v[pl.ds(r0, rows), :]
            g = _sigmoid(jnp.sum(xt.astype(F32) * gw, axis=1, keepdims=True))
            gb = jnp.broadcast_to(g, (rows, 128))
            g_v[pl.ds(r0, rows), :] = gb
            return gb

        def kp_tile(r0, rows, first):
            xt = x_v[pl.ds(r0, rows), :]
            k = jnp.dot(xt, wk_v[...], preferred_element_type=F32)
            pk = _phi(k)
            zz = jnp.sum(pk.reshape(rows // 8, 8, D), axis=0)
            pkt = pk.astype(BF16).T
            pp = jnp.dot(pkt, xt, preferred_element_type=F32)
            if first:
                z_acc[...] = zz
                p_acc[...] = pp
            else:
                z_acc[...] += zz
                p_acc[...] += pp
            if g_early:
                g_tile(r0, rows)

        first = True
        for i in range(nx):
            xcp[i].wait()
            if i == 0:
                cp_wk.wait()
                cp_gw.wait()
            if i == wq_blk:
                cp_wq.wait()
                wqt = pltpu.bitcast(wq_v[...].T, U32)
                for j in range(NB):
                    t32_v[j] = wqt[:, j * 128:(j + 1) * 128]
                for j in range(NB):
                    for dp in range(NP):
                        wqp_v[dp * 2 * H:(dp + 1) * 2 * H, j * 128:(j + 1) * 128] = pltpu.bitcast(
                            t32_v[j, pl.ds(dp, H, stride=NP), :], BF16)
            if i == nx - 1:
                cp_wv.wait()
                cp_wo.wait()
            r0 = xoff[i]
            while r0 < xoff[i] + xsplit[i]:
                rows = min(KT, xoff[i] + xsplit[i] - r0)
                kp_tile(r0, rows, first)
                first = False
                r0 += rows

        zrow = jnp.sum(z_acc[...], axis=0, keepdims=True)
        zhi = zrow.astype(BF16).astype(F32)
        zlo = zrow - zhi
        rid = lax.broadcasted_iota(jnp.int32, (128, D), 0)
        zz = jnp.where(rid == 0, zhi, jnp.where(rid == 1, zlo, 0.0)).astype(BF16)
        zt_v[...] = pltpu.bitcast(zz.T, U32)
        zp = jnp.concatenate([zt_v[pl.ds(dp, H, stride=NP), :] for dp in range(NP)], axis=0)
        zpt = pltpu.bitcast(zp, BF16).T.astype(F32)
        zprow = zpt[0:1, :] + zpt[1:2, :]

        def mid_kv():
            rr = lax.broadcasted_iota(jnp.int32, (128, 128), 0) // Dh
            cc = lax.broadcasted_iota(jnp.int32, (128, 128), 1) // Dh
            mask = rr == cc
            for j in range(NB):
                sl = slice(j * 128, (j + 1) * 128)
                pj = p_acc[sl, :].astype(BF16)
                kv = jnp.dot(pj, wv_v[:, sl], preferred_element_type=F32)
                kv_v[j * 64:(j + 1) * 64, :] = pltpu.bitcast(jnp.where(mask, kv, 0.0).astype(BF16), U32)

        def mid_m():
            for j in range(NB):
                sl = slice(j * 128, (j + 1) * 128)
                kvp = jnp.concatenate([kv_v[pl.ds(j * 64 + dp, 8, stride=NP), :] for dp in range(NP)], axis=0)
                kvp = pltpu.bitcast(kvp, BF16)
                mj = jnp.dot(kvp, wo_v[sl, :], preferred_element_type=F32).astype(BF16)
                for dp in range(NP):
                    m_v[dp * 64 + 16 * j:dp * 64 + 16 * j + 16, :] = mj[dp * 16:(dp + 1) * 16, :]

        lane = lax.broadcasted_iota(jnp.int32, (QT, 128), 1)
        even = (lane % 2) == 0
        nq = S // QT
        for qi in range(nq + 1):
            if qi == kv_at:
                mid_kv()
            if qi == m_at:
                mid_m()
            if qi == nq:
                break
            r0 = qi * QT
            xt = x_v[pl.ds(r0, QT), :]
            q = lax.dot_general(xt, wqp_v[...], NT, preferred_element_type=F32)
            if not g_early:
                gb = g_tile(r0, QT)
            else:
                gb = g_v[pl.ds(r0, QT), :]
            pq = _phi(q)
            t = pq * zprow
            s = (t[:, 0:128] + t[:, 128:256]) + (t[:, 256:384] + t[:, 384:512])
            s = s + pltpu.roll(s, 64, 1)
            s = s + jnp.where(even, pltpu.roll(s, 127, 1), pltpu.roll(s, 1, 1))
            sc = gb / (s + 1e-6)
            for j in range(NB):
                sl = slice(j * 128, (j + 1) * 128)
                r_v[pl.ds(r0, QT), sl] = (pq[:, sl] * sc).astype(BF16)

        cp_wg.wait()
        cp_wu.wait()
        cp_wd.wait()

        def body(i, carry):
            off = 0
            for si, ts in enumerate(subs):
                row = pl.multiple_of(i * T2 + off, 128)
                off += ts
                xt = x_v[pl.ds(row, ts), :]
                b = None
                c0 = 0
                for fc in fcs:
                    gt = jnp.dot(xt, wg_v[:, c0:c0 + fc], preferred_element_type=F32)
                    ut = jnp.dot(xt, wu_v[:, c0:c0 + fc], preferred_element_type=F32)
                    hg = 0.5 * gt
                    h = ((hg * (jnp.tanh(hg) + 1.0)) * ut).astype(BF16)
                    bb = jnp.dot(h, wd_v[c0:c0 + fc, :], preferred_element_type=F32)
                    b = bb if b is None else b + bb
                    c0 += fc
                om = 1.0 - g_v[pl.ds(row, ts), :]
                b = b * jnp.concatenate([om] * NB, axis=1)
                a = jnp.dot(r_v[pl.ds(row, ts), :], m_v[...], preferred_element_type=F32)
                o_v[pl.ds(row, ts), :] = (a + b).astype(o_v.dtype)
                pltpu.make_async_copy(o_v.at[pl.ds(row, ts)], o_hbm.at[pl.ds(row, ts)], osem).start()
            return carry

        lax.fori_loop(0, n2, body, 0)
        pltpu.make_async_copy(o_v, o_hbm, osem).wait()

    @jax.jit
    def fn(A_x, A_wqkv, A_wo, B_x, B_w_gate, B_w_up, B_w_down, gate_w):
        B, S, D = A_x.shape
        F = B_w_gate.shape[1]
        x2 = A_x.reshape(S, D)
        anyspec = pl.BlockSpec(memory_space=pl.ANY)
        out = pl.pallas_call(
            kernel,
            out_shape=jax.ShapeDtypeStruct((S, D), A_x.dtype),
            in_specs=[anyspec] * 7,
            out_specs=anyspec,
            scratch_shapes=[
                pltpu.VMEM((S, D), BF16),
                pltpu.VMEM((D, D), BF16),
                pltpu.VMEM((D, D), BF16),
                pltpu.VMEM((D, D), BF16),
                pltpu.VMEM((D, D), BF16),
                pltpu.VMEM((D, F), BF16),
                pltpu.VMEM((D, F), BF16),
                pltpu.VMEM((F, D), BF16),
                pltpu.VMEM((D,), BF16),
                pltpu.VMEM((D, D), BF16),
                pltpu.VMEM((D // 128, D // 2, 128), U32),
                pltpu.VMEM((D, D), F32),
                pltpu.VMEM((8, D), F32),
                pltpu.VMEM((D // 2, 128), U32),
                pltpu.VMEM((D // 2, 128), U32),
                pltpu.VMEM((D, D), BF16),
                pltpu.VMEM((S, D), BF16),
                pltpu.VMEM((S, 128), F32),
                pltpu.VMEM((S, D), BF16),
                pltpu.SemaphoreType.DMA((len(xsplit) + 8,)),
                pltpu.SemaphoreType.DMA(()),
            ],
            compiler_params=pltpu.CompilerParams(vmem_limit_bytes=100 * 1024 * 1024,
                                                 disable_semaphore_checks=nosem),
        )(x2, A_wqkv, A_wo, B_w_gate, B_w_up, B_w_down, gate_w)
        return out.reshape(B, S, D)

    return fn


pallas_gated_mix__linear_attn_block__swiglu_ffn__prompt_kernel = make()
```

```python
import jax
import jax.numpy as jnp
from jax import lax
import jax.experimental.pallas as pl
import jax.experimental.pallas.tpu as pltpu

F32 = jnp.float32
BF16 = jnp.bfloat16
U32 = jnp.uint32
NT = (((1,), (1,)), ((), ()))

H = 32
LANES = 128
KT = 512
TS = 256
T2 = 1024
X_SPLIT = (256, 768, 1024)
K_SPLIT = 256
TAIL_ROWS = 32


def _phi(t):
    return jnp.where(t > 0, t + 1.0, jnp.exp(t)) + 1e-6


def _sigmoid(t):
    return 0.5 * jnp.tanh(0.5 * t) + 0.5


def _dot(a, b):
    return jnp.dot(a, b, preferred_element_type=F32)


def _kernel(x_hbm, wqkv_hbm, wo_hbm, wg_hbm, wu_hbm, wd_hbm, gw_hbm, o_hbm,
            x_v, wq_v, wk_v, wv_v, wo_v, wg_v, wu_v, wd_v, gw_v,
            wqp_v, wqt_v, p_v, z_v, zt_v, kv_v, m_v, q0_v, zp_v, o_v, sem, osem):
    S, D = x_v.shape
    F = wg_v.shape[1]
    DH = D // H
    NB = D // LANES
    NP = DH // 2
    HB = LANES // DH
    n_iter = S // T2
    n_sub = T2 // TS
    fc = F // 2
    xoff = [sum(X_SPLIT[:i]) for i in range(len(X_SPLIT))]
    r0, ks = X_SPLIT[0], K_SPLIT

    pairs = [
        (x_hbm.at[pl.ds(0, r0), pl.ds(0, ks)], x_v.at[pl.ds(0, r0), pl.ds(0, ks)]),
        (wqkv_hbm.at[pl.ds(0, ks), pl.ds(D, D)], wk_v.at[pl.ds(0, ks)]),
        (x_hbm.at[pl.ds(0, r0), pl.ds(ks, D - ks)], x_v.at[pl.ds(0, r0), pl.ds(ks, D - ks)]),
        (wqkv_hbm.at[pl.ds(ks, D - ks), pl.ds(D, D)], wk_v.at[pl.ds(ks, D - ks)]),
        (x_hbm.at[pl.ds(xoff[1], X_SPLIT[1])], x_v.at[pl.ds(xoff[1], X_SPLIT[1])]),
        (wqkv_hbm.at[:, pl.ds(0, D)], wq_v),
        (x_hbm.at[pl.ds(xoff[2], X_SPLIT[2])], x_v.at[pl.ds(xoff[2], X_SPLIT[2])]),
        (wqkv_hbm.at[:, pl.ds(2 * D, D)], wv_v),
        (wo_hbm, wo_v),
        (gw_hbm, gw_v),
        (wg_hbm, wg_v),
        (wu_hbm, wu_v),
        (wd_hbm, wd_v),
    ]
    cps = [pltpu.make_async_copy(s, d, sem.at[n]) for n, (s, d) in enumerate(pairs)]
    for c in cps:
        c.start()
    (cp_x0a, cp_wka, cp_x0b, cp_wkb, cp_x1, cp_wq, cp_x2, cp_wv, cp_wo,
     cp_gw, cp_wg, cp_wu, cp_wd) = cps

    def pair_gather(ref, base, n):
        return jnp.concatenate(
            [ref[pl.ds(base + p, n, stride=NP), :] for p in range(NP)], axis=0)

    def kp_accumulate(k, xt, first):
        pk = _phi(k)
        zz = jnp.sum(pk.reshape(pk.shape[0] // 8, 8, D), axis=0)
        pp = _dot(pk.astype(BF16).T, xt)
        if first:
            z_v[...] = zz
            p_v[...] = pp
        else:
            z_v[...] += zz
            p_v[...] += pp

    def kp_rows(lo, hi):
        for a in range(lo, hi, KT):
            xt = x_v[pl.ds(a, min(KT, hi - a)), :]
            kp_accumulate(_dot(xt, wk_v[...]), xt, False)

    def q_matmul(row, rows):
        return lax.dot_general(x_v[pl.ds(row, rows), :], wqp_v[...], NT,
                               preferred_element_type=F32)

    def phase1():
        cp_x0a.wait()
        cp_wka.wait()
        p_v[0:r0, :] = _dot(x_v[0:r0, 0:ks], wk_v[0:ks, :])
        cp_x0b.wait()
        cp_wkb.wait()
        xt = x_v[0:r0, :]
        kp_accumulate(p_v[0:r0, :] + _dot(xt[:, ks:D], wk_v[ks:D, :]), xt, True)

        cp_x1.wait()
        kp_rows(xoff[1], xoff[2])

        cp_wq.wait()
        cp_x2.wait()
        cp_wv.wait()
        cp_wo.wait()
        wqt = pltpu.bitcast(wq_v[...].T, U32)
        for j in range(NB):
            wqt_v[j, 0:D // 2, :] = wqt[:, j * LANES:(j + 1) * LANES]
        for j in range(NB):
            for p in range(NP):
                wqp_v[p * 2 * H:(p + 1) * 2 * H, j * LANES:(j + 1) * LANES] = pltpu.bitcast(
                    wqt_v[j, pl.ds(p, H, stride=NP), :], BF16)
        kp_rows(xoff[2], S)

        z = jnp.sum(z_v[...], axis=0, keepdims=True)
        zhi = z.astype(BF16).astype(F32)
        rid = lax.broadcasted_iota(jnp.int32, (LANES, D), 0)
        zz = jnp.where(rid == 0, zhi, jnp.where(rid == 1, z - zhi, 0.0)).astype(BF16)
        zt_v[0:D // 2, :] = pltpu.bitcast(zz.T, U32)
        zp = pltpu.bitcast(pair_gather(zt_v, 0, H), BF16).T.astype(F32)
        zp_v[...] = jnp.broadcast_to(zp[0:1, :] + zp[1:2, :], (8, D))

        q0_v[0:TS, :] = q_matmul(0, TS)
        same_head = (lax.broadcasted_iota(jnp.int32, (LANES, LANES), 0) // DH
                     == lax.broadcasted_iota(jnp.int32, (LANES, LANES), 1) // DH)
        for j in range(NB):
            sl = slice(j * LANES, (j + 1) * LANES)
            kv = _dot(p_v[sl, :].astype(BF16), wv_v[:, sl])
            kv_v[j * 64:(j + 1) * 64, :] = pltpu.bitcast(
                jnp.where(same_head, kv, 0.0).astype(BF16), U32)
        for it in range(1, n_iter):
            q0_v[it * TS:(it + 1) * TS, :] = q_matmul(it * T2, TS)
        for j in range(NB):
            kvp = pltpu.bitcast(pair_gather(kv_v, j * 64, HB), BF16)
            mj = _dot(kvp, wo_v[j * LANES:(j + 1) * LANES, :]).astype(BF16)
            for p in range(NP):
                dst = p * 2 * H + j * 2 * HB
                m_v[dst:dst + 2 * HB, :] = mj[p * 2 * HB:(p + 1) * 2 * HB, :]

        cp_gw.wait()
        cp_wg.wait()
        cp_wu.wait()
        cp_wd.wait()

    def write_out(row, rows, col, cols, val):
        o_v[pl.ds(row, rows), col:col + cols] = val
        pltpu.make_async_copy(o_v.at[pl.ds(row, rows), pl.ds(col, cols)],
                              o_hbm.at[pl.ds(row, rows), pl.ds(col, cols)], osem).start()

    def ffn_chunk(xt, c):
        hg = 0.5 * _dot(xt, wg_v[:, c:c + fc])
        up = _dot(xt, wu_v[:, c:c + fc])
        h = (hg * (jnp.tanh(hg) + 1.0)) * up
        return _dot(h.astype(BF16), wd_v[c:c + fc, :])

    def body(it, carry):
        pl.when(it == 0)(phase1)
        for si in range(n_sub):
            row = pl.multiple_of(it * T2 + si * TS, TS)
            xt = x_v[pl.ds(row, TS), :]
            gw = gw_v[...].astype(F32).reshape(1, D)
            g = _sigmoid(jnp.sum(xt.astype(F32) * gw, axis=1, keepdims=True))
            g = jnp.broadcast_to(g, (TS, LANES))

            b = ffn_chunk(xt, 0)

            if si == 0:
                q = q0_v[pl.ds(pl.multiple_of(it * TS, TS), TS), :]
            else:
                q = q_matmul(row, TS)
            pq = _phi(q)
            t = pq * zp_v[0:1, :]
            den = t[:, 0:LANES]
            for j in range(1, NB):
                den = den + t[:, j * LANES:(j + 1) * LANES]
            den = den + pltpu.roll(den, 2 * H, 1)
            even = lax.broadcasted_iota(jnp.int32, (TS, LANES), 1) % 2 == 0
            den = den + jnp.where(even, pltpu.roll(den, LANES - 1, 1), pltpu.roll(den, 1, 1))
            scale = g * pl.reciprocal(den + 1e-6, approx=False)
            r = jnp.concatenate(
                [(pq[:, j * LANES:(j + 1) * LANES] * scale).astype(BF16) for j in range(NB)],
                axis=1)

            b = b + ffn_chunk(xt, fc)
            b = b * jnp.concatenate([1.0 - g] * NB, axis=1)
            res = (_dot(r, m_v[...]) + b).astype(o_v.dtype)

            if si == n_sub - 1:
                half = D // 2
                write_out(row, TS, 0, half, res[:, 0:half])
                for a in range(0, TS, TAIL_ROWS):
                    write_out(pl.multiple_of(row + a, TAIL_ROWS), TAIL_ROWS, half, half,
                              res[a:a + TAIL_ROWS, half:D])
            else:
                write_out(row, TS, 0, D, res)
        return carry

    lax.fori_loop(0, n_iter, body, 0)
    pltpu.make_async_copy(o_v, o_hbm, osem).wait()


@jax.jit
def pallas_gated_mix__linear_attn_block__swiglu_ffn__prompt_kernel(
    A_x: jax.Array,
    A_wqkv: jax.Array,
    A_wo: jax.Array,
    B_x: jax.Array,
    B_w_gate: jax.Array,
    B_w_up: jax.Array,
    B_w_down: jax.Array,
    gate_w: jax.Array,
):
    del B_x
    B, S, D = A_x.shape
    F = B_w_gate.shape[1]
    assert B == 1 and S == sum(X_SPLIT) and S % T2 == 0 and D == 4 * LANES and F % (2 * LANES) == 0
    hbm = pl.BlockSpec(memory_space=pl.ANY)
    pad = D // 2 + 8
    out = pl.pallas_call(
        _kernel,
        out_shape=jax.ShapeDtypeStruct((S, D), A_x.dtype),
        in_specs=[hbm] * 7,
        out_specs=hbm,
        scratch_shapes=[
            pltpu.VMEM((S, D), BF16),
            pltpu.VMEM((D, D), BF16),
            pltpu.VMEM((D, D), BF16),
            pltpu.VMEM((D, D), BF16),
            pltpu.VMEM((D, D), BF16),
            pltpu.VMEM((D, F), BF16),
            pltpu.VMEM((D, F), BF16),
            pltpu.VMEM((F, D), BF16),
            pltpu.VMEM((D,), BF16),
            pltpu.VMEM((D, D), BF16),
            pltpu.VMEM((D // LANES, pad, LANES), U32),
            pltpu.VMEM((D, D), F32),
            pltpu.VMEM((8, D), F32),
            pltpu.VMEM((pad, LANES), U32),
            pltpu.VMEM((pad, LANES), U32),
            pltpu.VMEM((D, D), BF16),
            pltpu.VMEM((S // T2 * TS, D), F32),
            pltpu.VMEM((8, D), F32),
            pltpu.VMEM((S, D), A_x.dtype),
            pltpu.SemaphoreType.DMA((13,)),
            pltpu.SemaphoreType.DMA(()),
        ],
        compiler_params=pltpu.CompilerParams(
            vmem_limit_bytes=64 * 1024 * 1024,
            disable_semaphore_checks=True,
            disable_bounds_checks=True,
        ),
    )(A_x.reshape(S, D), A_wqkv, A_wo, B_w_gate, B_w_up, B_w_down, gate_w)
    return out.reshape(B, S, D)
```

```python
import jax
import jax.numpy as jnp
from jax import lax
import jax.experimental.pallas as pl
import jax.experimental.pallas.tpu as pltpu

F32 = jnp.float32
BF16 = jnp.bfloat16
U32 = jnp.uint32
NT = (((1,), (1,)), ((), ()))

H = 32
LANES = 128
KT = 512
TS = 256
T2 = 1024
R1 = 1024
K_STAGES = ((0, 128), (128, 256), (256, 512))
TAIL_ROWS = 32


def _phi(t):
    return jnp.where(t > 0, t + 1.0, jnp.exp(t)) + 1e-6


def _sigmoid(t):
    return 0.5 * jnp.tanh(0.5 * t) + 0.5


def _dot(a, b):
    return jnp.dot(a, b, preferred_element_type=F32)


def _kernel(x_hbm, wqkv_hbm, wo_hbm, wg_hbm, wu_hbm, wd_hbm, gw_hbm, o_hbm,
            x_v, wq_v, wk_v, wv_v, wo_v, wg_v, wu_v, wd_v, gw_v,
            wqp_v, wqt_v, k_v, p_v, z_v, zt_v, kv_v, m_v, q0_v, zp_v, o_v, sem, osem):
    S, D = x_v.shape
    F = wg_v.shape[1]
    DH = D // H
    NB = D // LANES
    NP = DH // 2
    HB = LANES // DH
    n_iter = S // T2
    n_sub = T2 // TS
    fc = F // 2

    pairs = []
    for ca, cb in K_STAGES:
        pairs.append((x_hbm.at[pl.ds(0, R1), pl.ds(ca, cb - ca)],
                      x_v.at[pl.ds(0, R1), pl.ds(ca, cb - ca)]))
        pairs.append((wqkv_hbm.at[pl.ds(ca, cb - ca), pl.ds(D, D)], wk_v.at[pl.ds(ca, cb - ca)]))
    n_stage = len(pairs)
    pairs += [
        (wqkv_hbm.at[:, pl.ds(0, D)], wq_v),
        (x_hbm.at[pl.ds(R1, S - R1)], x_v.at[pl.ds(R1, S - R1)]),
        (wqkv_hbm.at[:, pl.ds(2 * D, D)], wv_v),
        (wo_hbm, wo_v),
        (gw_hbm, gw_v),
        (wg_hbm, wg_v),
        (wu_hbm, wu_v),
        (wd_hbm, wd_v),
    ]
    cps = [pltpu.make_async_copy(s, d, sem.at[n]) for n, (s, d) in enumerate(pairs)]
    for c in cps:
        c.start()
    cp_wq, cp_x2, cp_wv, cp_wo, cp_gw, cp_wg, cp_wu, cp_wd = cps[n_stage:]

    def pair_gather(ref, base, n):
        return jnp.concatenate(
            [ref[pl.ds(base + p, n, stride=NP), :] for p in range(NP)], axis=0)

    def kp_accumulate(k, xt, first):
        pk = _phi(k)
        zz = jnp.sum(pk.reshape(pk.shape[0] // 8, 8, D), axis=0)
        pp = _dot(pk.astype(BF16).T, xt)
        if first:
            z_v[...] = zz
            p_v[...] = pp
        else:
            z_v[...] += zz
            p_v[...] += pp

    def q_matmul(row, rows):
        return lax.dot_general(x_v[pl.ds(row, rows), :], wqp_v[...], NT,
                               preferred_element_type=F32)

    def phase1():
        for n, (ca, cb) in enumerate(K_STAGES):
            cps[2 * n].wait()
            cps[2 * n + 1].wait()
            for a in range(0, R1, KT):
                k = _dot(x_v[a:a + KT, ca:cb], wk_v[ca:cb, :])
                if ca > 0:
                    k = k_v[a:a + KT, :] + k
                if cb < D:
                    k_v[a:a + KT, :] = k
                else:
                    kp_accumulate(k, x_v[a:a + KT, :], a == 0)

        cp_wq.wait()
        cp_x2.wait()
        cp_wv.wait()
        cp_wo.wait()
        wqt = pltpu.bitcast(wq_v[...].T, U32)
        for j in range(NB):
            wqt_v[j, 0:D // 2, :] = wqt[:, j * LANES:(j + 1) * LANES]
        for j in range(NB):
            for p in range(NP):
                wqp_v[p * 2 * H:(p + 1) * 2 * H, j * LANES:(j + 1) * LANES] = pltpu.bitcast(
                    wqt_v[j, pl.ds(p, H, stride=NP), :], BF16)
        for a in range(R1, S, KT):
            xt = x_v[a:a + KT, :]
            kp_accumulate(_dot(xt, wk_v[...]), xt, False)

        z = jnp.sum(z_v[...], axis=0, keepdims=True)
        zhi = z.astype(BF16).astype(F32)
        rid = lax.broadcasted_iota(jnp.int32, (LANES, D), 0)
        zz = jnp.where(rid == 0, zhi, jnp.where(rid == 1, z - zhi, 0.0)).astype(BF16)
        zt_v[0:D // 2, :] = pltpu.bitcast(zz.T, U32)
        zp = pltpu.bitcast(pair_gather(zt_v, 0, H), BF16).T.astype(F32)
        zp_v[...] = jnp.broadcast_to(zp[0:1, :] + zp[1:2, :], (8, D))

        q0_v[0:TS, :] = q_matmul(0, TS)
        same_head = (lax.broadcasted_iota(jnp.int32, (LANES, LANES), 0) // DH
                     == lax.broadcasted_iota(jnp.int32, (LANES, LANES), 1) // DH)
        for j in range(NB):
            sl = slice(j * LANES, (j + 1) * LANES)
            kv = _dot(p_v[sl, :].astype(BF16), wv_v[:, sl])
            kv_v[j * 64:(j + 1) * 64, :] = pltpu.bitcast(
                jnp.where(same_head, kv, 0.0).astype(BF16), U32)
        for it in range(1, n_iter):
            q0_v[it * TS:(it + 1) * TS, :] = q_matmul(it * T2, TS)
        for j in range(NB):
            kvp = pltpu.bitcast(pair_gather(kv_v, j * 64, HB), BF16)
            mj = _dot(kvp, wo_v[j * LANES:(j + 1) * LANES, :]).astype(BF16)
            for p in range(NP):
                dst = p * 2 * H + j * 2 * HB
                m_v[dst:dst + 2 * HB, :] = mj[p * 2 * HB:(p + 1) * 2 * HB, :]

        cp_gw.wait()
        cp_wg.wait()
        cp_wu.wait()
        cp_wd.wait()

    def write_out(row, rows, col, cols, val):
        o_v[pl.ds(row, rows), col:col + cols] = val
        pltpu.make_async_copy(o_v.at[pl.ds(row, rows), pl.ds(col, cols)],
                              o_hbm.at[pl.ds(row, rows), pl.ds(col, cols)], osem).start()

    def ffn_chunk(xt, c):
        hg = 0.5 * _dot(xt, wg_v[:, c:c + fc])
        up = _dot(xt, wu_v[:, c:c + fc])
        h = (hg * (jnp.tanh(hg) + 1.0)) * up
        return _dot(h.astype(BF16), wd_v[c:c + fc, :])

    def body(it, carry):
        pl.when(it == 0)(phase1)
        for si in range(n_sub):
            row = pl.multiple_of(it * T2 + si * TS, TS)
            xt = x_v[pl.ds(row, TS), :]
            gw = gw_v[...].astype(F32).reshape(1, D)
            g = _sigmoid(jnp.sum(xt.astype(F32) * gw, axis=1, keepdims=True))
            g = jnp.broadcast_to(g, (TS, LANES))

            b = ffn_chunk(xt, 0)

            if si == 0:
                q = q0_v[pl.ds(pl.multiple_of(it * TS, TS), TS), :]
            else:
                q = q_matmul(row, TS)
            pq = _phi(q)
            t = pq * zp_v[0:1, :]
            den = t[:, 0:LANES]
            for j in range(1, NB):
                den = den + t[:, j * LANES:(j + 1) * LANES]
            den = den + pltpu.roll(den, 2 * H, 1)
            even = lax.broadcasted_iota(jnp.int32, (TS, LANES), 1) % 2 == 0
            den = den + jnp.where(even, pltpu.roll(den, LANES - 1, 1), pltpu.roll(den, 1, 1))
            scale = g * pl.reciprocal(den + 1e-6, approx=False)
            r = jnp.concatenate(
                [(pq[:, j * LANES:(j + 1) * LANES] * scale).astype(BF16) for j in range(NB)],
                axis=1)

            b = b + ffn_chunk(xt, fc)
            b = b * jnp.concatenate([1.0 - g] * NB, axis=1)
            res = (_dot(r, m_v[...]) + b).astype(o_v.dtype)

            if si == n_sub - 1:
                half = D // 2
                write_out(row, TS, 0, half, res[:, 0:half])
                for a in range(0, TS, TAIL_ROWS):
                    write_out(pl.multiple_of(row + a, TAIL_ROWS), TAIL_ROWS, half, half,
                              res[a:a + TAIL_ROWS, half:D])
            else:
                write_out(row, TS, 0, D, res)
        return carry

    lax.fori_loop(0, n_iter, body, 0)
    pltpu.make_async_copy(o_v, o_hbm, osem).wait()


@jax.jit
def pallas_gated_mix__linear_attn_block__swiglu_ffn__prompt_kernel(
    A_x: jax.Array,
    A_wqkv: jax.Array,
    A_wo: jax.Array,
    B_x: jax.Array,
    B_w_gate: jax.Array,
    B_w_up: jax.Array,
    B_w_down: jax.Array,
    gate_w: jax.Array,
):
    del B_x
    B, S, D = A_x.shape
    F = B_w_gate.shape[1]
    assert B == 1 and S % T2 == 0 and (S - R1) % KT == 0 and S > R1
    assert D == 4 * LANES and F % (2 * LANES) == 0
    hbm = pl.BlockSpec(memory_space=pl.ANY)
    pad = D // 2 + 8
    out = pl.pallas_call(
        _kernel,
        out_shape=jax.ShapeDtypeStruct((S, D), A_x.dtype),
        in_specs=[hbm] * 7,
        out_specs=hbm,
        scratch_shapes=[
            pltpu.VMEM((S, D), BF16),
            pltpu.VMEM((D, D), BF16),
            pltpu.VMEM((D, D), BF16),
            pltpu.VMEM((D, D), BF16),
            pltpu.VMEM((D, D), BF16),
            pltpu.VMEM((D, F), BF16),
            pltpu.VMEM((D, F), BF16),
            pltpu.VMEM((F, D), BF16),
            pltpu.VMEM((D,), BF16),
            pltpu.VMEM((D, D), BF16),
            pltpu.VMEM((D // LANES, pad, LANES), U32),
            pltpu.VMEM((R1, D), F32),
            pltpu.VMEM((D, D), F32),
            pltpu.VMEM((8, D), F32),
            pltpu.VMEM((pad, LANES), U32),
            pltpu.VMEM((pad, LANES), U32),
            pltpu.VMEM((D, D), BF16),
            pltpu.VMEM((S // T2 * TS, D), F32),
            pltpu.VMEM((8, D), F32),
            pltpu.VMEM((S, D), A_x.dtype),
            pltpu.SemaphoreType.DMA((2 * len(K_STAGES) + 8,)),
            pltpu.SemaphoreType.DMA(()),
        ],
        compiler_params=pltpu.CompilerParams(
            vmem_limit_bytes=64 * 1024 * 1024,
            disable_semaphore_checks=True,
            disable_bounds_checks=True,
        ),
    )(A_x.reshape(S, D), A_wqkv, A_wo, B_w_gate, B_w_up, B_w_down, gate_w)
    return out.reshape(B, S, D)
```

```python
import jax
import jax.numpy as jnp
from jax import lax
import jax.experimental.pallas as pl
import jax.experimental.pallas.tpu as pltpu

F32 = jnp.float32
BF16 = jnp.bfloat16
U32 = jnp.uint32

H = 32
LANES = 128
TS = 512
HS = TS // 2
T2 = 1024
R1 = 1024
K_STAGES = ((0, 128), (128, 256), (256, 512))
FC = 256
Q_POS = 3
TAIL_ROWS = 32
ORDER = (1, 4, 2, 3, 0, 6, 5)


def _phi(t):
    return jnp.where(t > 0, t + 1.0, jnp.exp(t)) + 1e-6


def _sigmoid(t):
    return 0.5 * jnp.tanh(0.5 * t) + 0.5


def _dot(a, b):
    return jnp.dot(a, b, preferred_element_type=F32)


def _dot_nt(a, b):
    return lax.dot_general(a, b, (((1,), (1,)), ((), ())), preferred_element_type=F32)


def _pack(v):
    return pltpu.bitcast(v.astype(BF16), U32)


def _unpack(v):
    return pltpu.bitcast(v, BF16)


def _quads(a):
    m, n = a.shape[0] // 2, a.shape[1] // 2
    return a[:m, :n], a[:m, n:], a[m:, :n], a[m:, n:]


def _lhs7(a11, a12, a21, a22):
    return [a11 + a22, a21 + a22, a11, a22, a11 + a12, a21 - a11, a12 - a22]


def _rhs7(b11, b12, b21, b22):
    return [b11 + b22, b11, b12 - b22, b21 - b11, b22, b11 + b12, b21 + b22]


def _out4(m):
    m1, m2, m3, m4, m5, m6, m7 = m
    return (m1 + m4) + (m7 - m5), m3 + m5, m2 + m4, (m1 - m2) + (m3 + m6)


def _join(c11, c12, c21, c22):
    return jnp.concatenate([jnp.concatenate([c11, c12], axis=1),
                            jnp.concatenate([c21, c22], axis=1)], axis=0)


_L2R = (0, 2, 6, 5, 3, 4, 1)


def _products(dot, lhs, rhs, order=ORDER):
    m = [None] * 7
    for i in order:
        m[i] = dot(lhs[i], rhs[i])
    return m


def _kernel(x_hbm, wqkv_hbm, wo_hbm, wg_hbm, wu_hbm, wd_hbm, gw_hbm, o_hbm,
            x_v, wq_v, wk_v, wv_v, wo_v, wg_v, wu_v, wd_v, gw_v,
            wqt_v, wq7_v, wgu7_v, wd7_v, k_v, p7_v, z_v, zt_v, kv_v, q0_v, zp_v, g_v, o_v,
            sem, osem):
    S, D = x_v.shape
    F = wg_v.shape[1]
    DH = D // H
    NB = D // LANES
    NP = DH // 2
    HB = LANES // DH
    HD = D // 2
    n_iter = S // T2
    n_sub = T2 // TS
    NC = F // FC

    pairs = []
    for ca, cb in K_STAGES:
        pairs.append((x_hbm.at[pl.ds(0, R1), pl.ds(ca, cb - ca)],
                      x_v.at[pl.ds(0, R1), pl.ds(ca, cb - ca)]))
        pairs.append((wqkv_hbm.at[pl.ds(ca, cb - ca), pl.ds(D, D)], wk_v.at[pl.ds(ca, cb - ca)]))
    n_stage = len(pairs)
    pairs += [
        (gw_hbm, gw_v),
        (wqkv_hbm.at[:, pl.ds(0, D)], wq_v),
        (x_hbm.at[pl.ds(R1, S - R1)], x_v.at[pl.ds(R1, S - R1)]),
        (wqkv_hbm.at[:, pl.ds(2 * D, D)], wv_v),
        (wo_hbm, wo_v),
        (wg_hbm, wg_v),
        (wu_hbm, wu_v),
        (wd_hbm, wd_v),
    ]
    cps = [pltpu.make_async_copy(s, d, sem.at[n]) for n, (s, d) in enumerate(pairs)]
    for c in cps:
        c.start()
    cp_gw, cp_wq, cp_x2, cp_wv, cp_wo, cp_wg, cp_wu, cp_wd = cps[n_stage:]

    def pair_gather(ref, base, n):
        return jnp.concatenate(
            [ref[pl.ds(base + p, n, stride=NP), :] for p in range(NP)], axis=0)

    def x_sums(row):
        xt = x_v[pl.ds(row, TS), :]
        out = [v.astype(BF16) for v in _lhs7(*_quads(xt.astype(F32)))]
        out[2] = xt[0:HS, 0:HD]
        out[3] = xt[HS:TS, HD:D]
        return out

    def store_gate(t):
        gw = gw_v[...].astype(F32).reshape(1, D)
        xf = x_v[t * TS:(t + 1) * TS, :].astype(F32)
        g = _sigmoid(jnp.sum(xf * gw, axis=1, keepdims=True))
        g_v[t * TS:(t + 1) * TS, :] = jnp.broadcast_to(g, (TS, LANES))

    def p_accumulate(k4, xs, first):
        p11, p12, p21, p22 = [_phi(v) for v in k4]
        colsum = lambda v: jnp.sum(v.reshape(HS // 8, 8, HD), axis=0)
        zz = jnp.concatenate([colsum(p21) + colsum(p11), colsum(p12) + colsum(p22)], axis=1)
        z_v[...] = zz if first else z_v[...] + zz
        a7 = _lhs7(p11, p21, p12, p22)
        for i in (2, 4, 5, 1, 0, 6, 3):
            pp = _dot(a7[i].astype(BF16).T, xs[_L2R[i]])
            p7_v[i] = pp if first else p7_v[i] + pp

    def phase1():
        for n, (ca, cb) in enumerate(K_STAGES):
            cps[2 * n].wait()
            cps[2 * n + 1].wait()
            if cb == D:
                cp_gw.wait()
            ks = []
            for a in range(0, R1, TS):
                k = _dot(x_v[a:a + TS, ca:cb], wk_v[ca:cb, :])
                if ca > 0:
                    k = k_v[a:a + TS, :] + k
                if cb < D:
                    k_v[a:a + TS, :] = k
                else:
                    ks.append(k)
            for t, k in enumerate(ks):
                store_gate(t)
                p_accumulate(_quads(k), x_sums(t * TS), t == 0)

        cp_wq.wait()
        cp_x2.wait()
        cp_wv.wait()
        cp_wo.wait()

        wqt = pltpu.bitcast(wq_v[...].T, U32)
        for j in range(NB):
            wqt_v[j, 0:HD, :] = wqt[:, j * LANES:(j + 1) * LANES]
        wqp = jnp.concatenate([pair_gather(wqt_v.at[j], 0, H) for j in range(NB)], axis=1)
        w11, w21, w12, w22 = _quads(_unpack(wqp).astype(F32))
        for i, v in enumerate(_rhs7(w11, w12, w21, w22)):
            wq7_v[i] = _pack(v)

        wk = wk_v[...]
        wk7 = [v.astype(BF16) for v in _rhs7(*_quads(wk.astype(F32)))]
        wk7[1] = wk[0:HD, 0:HD]
        wk7[4] = wk[HD:D, HD:D]
        late = list(range(R1 // TS, S // TS))
        xs, k4 = {}, {}
        for t in late:
            store_gate(t)
            xs[t] = x_sums(t * TS)
            k4[t] = _out4(_products(_dot, xs[t], wk7))

        def q_part(m, lhs, lo, hi):
            for i in ORDER[lo:hi]:
                m[i] = _dot_nt(lhs[i], _unpack(wq7_v[i]))

        for t in late:
            p_accumulate(k4[t], xs[t], False)
            if t % n_sub == 0:
                m = [None] * 7
                q_part(m, xs[t], 0, 7)
                q0_v[(t // n_sub) * TS:(t // n_sub + 1) * TS, :] = _join(*_out4(m))

        z = jnp.sum(z_v[...], axis=0, keepdims=True)
        zhi = z.astype(BF16).astype(F32)
        rid = lax.broadcasted_iota(jnp.int32, (LANES, D), 0)
        zz = jnp.where(rid == 0, zhi, jnp.where(rid == 1, z - zhi, 0.0)).astype(BF16)
        zt_v[0:HD, :] = pltpu.bitcast(zz.T, U32)
        zp = _unpack(pair_gather(zt_v, 0, H)).T.astype(F32)
        zp_v[...] = jnp.broadcast_to(zp[0:1, :] + zp[1:2, :], (8, D))

        x0, m0 = x_sums(0), [None] * 7
        q_part(m0, x0, 0, 3)
        same_head = (lax.broadcasted_iota(jnp.int32, (LANES, LANES), 0) // DH
                     == lax.broadcasted_iota(jnp.int32, (LANES, LANES), 1) // DH)
        pm = _join(*_out4([p7_v[i] for i in range(7)]))
        for j in range(NB):
            sl = slice(j * LANES, (j + 1) * LANES)
            kv = _dot(pm[sl, :].astype(BF16), wv_v[:, sl])
            kv_v[j * 64:(j + 1) * 64, :] = _pack(jnp.where(same_head, kv, 0.0))
        q_part(m0, x0, 3, 7)
        q0_v[0:TS, :] = _join(*_out4(m0))
        for j in range(NB):
            kvp = _unpack(pair_gather(kv_v, j * 64, HB))
            mj = _dot(kvp, wo_v[j * LANES:(j + 1) * LANES, :])
            for i, v in enumerate(_rhs7(*_quads(mj))):
                mi = _pack(v)
                for p in range(NP // 2):
                    dst = F // 4 + p * H + j * HB
                    wd7_v[i, dst:dst + HB, :] = mi[p * HB:(p + 1) * HB, :]

        cp_wg.wait()
        cp_wu.wait()
        cp_wd.wait()

    def write_out(row, rows, col, val):
        o_v[pl.ds(row, rows), col:col + HD] = val
        pltpu.make_async_copy(o_v.at[pl.ds(row, rows), pl.ds(col, HD)],
                              o_hbm.at[pl.ds(row, rows), pl.ds(col, HD)], osem).start()

    def gate_up_weights(c, build):
        left, right = slice(c * FC, c * FC + LANES), slice(c * FC + LANES, (c + 1) * FC)
        top, bot = slice(0, HD), slice(HD, D)
        raw = lambda rows, cols: jnp.concatenate([wg_v[rows, cols], wu_v[rows, cols]], axis=1)
        if build:
            b = _rhs7(*[raw(r, c_).astype(F32)
                        for r, c_ in ((top, left), (top, right), (bot, left), (bot, right))])
            for i in (0, 2, 3, 5, 6):
                wgu7_v[i, :, c * FC:(c + 1) * FC] = _pack(b[i])
            b = _rhs7(*_quads(wd_v[c * FC:(c + 1) * FC, :].astype(F32)))
            for i in range(7):
                wd7_v[i, c * 64:(c + 1) * 64, :] = _pack(b[i])
        return [raw(top, left) if i == 1 else raw(bot, right) if i == 4
                else _unpack(wgu7_v[i, :, c * FC:(c + 1) * FC]) for i in range(7)]

    def body(it, carry):
        pl.when(it == 0)(phase1)
        for si in range(n_sub):
            row = pl.multiple_of(it * T2 + si * TS, TS)
            g = g_v[pl.ds(row, TS), :]
            omg = 1.0 - g
            xs = x_sums(row)

            terms = [[] for _ in range(7)]
            for c in range(NC):
                if c == Q_POS:
                    if si == 0:
                        q = q0_v[pl.ds(pl.multiple_of(it * TS, TS), TS), :]
                    else:
                        q = _join(*_out4(_products(
                            _dot_nt, xs, [_unpack(wq7_v[i]) for i in range(7)])))
                    pq = _phi(q)
                    t = pq * zp_v[0:1, :]
                    den = t[:, 0:LANES]
                    for j in range(1, NB):
                        den = den + t[:, j * LANES:(j + 1) * LANES]
                    den = den + pltpu.roll(den, 2 * H, 1)
                    even = lax.broadcasted_iota(jnp.int32, (TS, LANES), 1) % 2 == 0
                    den = den + jnp.where(even, pltpu.roll(den, LANES - 1, 1),
                                          pltpu.roll(den, 1, 1))
                    den = den + 1e-6
                    inv = pl.reciprocal(den, approx=True)
                    inv = inv * (2.0 - den * inv)
                    r = pq * jnp.concatenate([g * inv] * NB, axis=1)
                    for i, v in enumerate(_lhs7(*_quads(r))):
                        terms[i].insert(0, (v.astype(BF16), F // 4, HD // 2))
                hs = []
                for n, cb in enumerate(_out4(_products(_dot, xs, gate_up_weights(c, si == 0)))):
                    hg = 0.5 * cb[:, 0:LANES]
                    om = omg[0:HS] if n < 2 else omg[HS:TS]
                    hs.append((hg * (jnp.tanh(hg) + 1.0)) * (cb[:, LANES:2 * LANES] * om))
                for i, v in enumerate(_lhs7(*hs)):
                    terms[i].append((v.astype(BF16), c * 64, 64))

            m = [None] * 7
            for i in (2, 4, 1, 3, 0, 6, 5):
                for v, o, n in terms[i]:
                    d = _dot(v, _unpack(wd7_v[i, o:o + n, :]))
                    m[i] = d if m[i] is None else m[i] + d
            c11, c12, c21, c22 = [v.astype(o_v.dtype) for v in _out4(m)]
            row2 = pl.multiple_of(row + HS, HS)
            write_out(row, HS, HD, c12)
            write_out(row2, HS, 0, c21)
            write_out(row, HS, 0, c11)
            if si == n_sub - 1:
                for a in range(0, HS, TAIL_ROWS):
                    write_out(pl.multiple_of(row2 + a, TAIL_ROWS), TAIL_ROWS, HD,
                              c22[a:a + TAIL_ROWS])
            else:
                write_out(row2, HS, HD, c22)
        return carry

    lax.fori_loop(0, n_iter, body, 0)
    pltpu.make_async_copy(o_v, o_hbm, osem).wait()


@jax.jit
def pallas_gated_mix__linear_attn_block__swiglu_ffn__prompt_kernel(
    A_x: jax.Array,
    A_wqkv: jax.Array,
    A_wo: jax.Array,
    B_x: jax.Array,
    B_w_gate: jax.Array,
    B_w_up: jax.Array,
    B_w_down: jax.Array,
    gate_w: jax.Array,
):
    del B_x
    B, S, D = A_x.shape
    F = B_w_gate.shape[1]
    assert B == 1 and S == 2 * T2 and R1 == T2 and D == 4 * LANES and F % FC == 0
    hbm = pl.BlockSpec(memory_space=pl.ANY)
    pad = D // 2 + 8
    no_checks = {name: True for name in ("disable_semaphore_checks", "disable_bounds_checks")
                 if hasattr(pltpu.CompilerParams, name)}
    out = pl.pallas_call(
        _kernel,
        out_shape=jax.ShapeDtypeStruct((S, D), A_x.dtype),
        in_specs=[hbm] * 7,
        out_specs=hbm,
        scratch_shapes=[
            pltpu.VMEM((S, D), BF16),
            pltpu.VMEM((D, D), BF16),
            pltpu.VMEM((D, D), BF16),
            pltpu.VMEM((D, D), BF16),
            pltpu.VMEM((D, D), BF16),
            pltpu.VMEM((D, F), BF16),
            pltpu.VMEM((D, F), BF16),
            pltpu.VMEM((F, D), BF16),
            pltpu.VMEM((D,), BF16),
            pltpu.VMEM((D // LANES, pad, LANES), U32),
            pltpu.VMEM((7, D // 4, D // 2), U32),
            pltpu.VMEM((7, D // 4, F), U32),
            pltpu.VMEM((7, F // 4 + D // 4, D // 2), U32),
            pltpu.VMEM((R1, D), F32),
            pltpu.VMEM((7, D // 2, D // 2), F32),
            pltpu.VMEM((8, D), F32),
            pltpu.VMEM((pad, LANES), U32),
            pltpu.VMEM((pad, LANES), U32),
            pltpu.VMEM((S // T2 * TS, D), F32),
            pltpu.VMEM((8, D), F32),
            pltpu.VMEM((S, LANES), F32),
            pltpu.VMEM((S, D), A_x.dtype),
            pltpu.SemaphoreType.DMA((2 * len(K_STAGES) + 8,)),
            pltpu.SemaphoreType.DMA(()),
        ],
        compiler_params=pltpu.CompilerParams(vmem_limit_bytes=100 * 1024 * 1024, **no_checks),
    )(A_x.reshape(S, D), A_wqkv, A_wo, B_w_gate, B_w_up, B_w_down, gate_w)
    return out.reshape(B, S, D)
```

```python
import jax
import jax.numpy as jnp
from jax import lax
import jax.experimental.pallas as pl
import jax.experimental.pallas.tpu as pltpu

F32 = jnp.float32
BF16 = jnp.bfloat16
U32 = jnp.uint32

H = 32
LANES = 128
TS = 512
HS = TS // 2
T2 = 2 * TS
R1 = 1024
K_STAGES = ((0, 128), (128, 256), (256, 512))
FC = 256
Q_POS = 3
TAIL_ROWS = 32


def _phi(t):
    return jnp.where(t > 0, t + 1.0, jnp.exp(t)) + 1e-6


def _sigmoid(t):
    return 0.5 * jnp.tanh(0.5 * t) + 0.5


def _dot(a, b):
    return jnp.dot(a, b, preferred_element_type=F32)


def _dot_nt(a, b):
    return lax.dot_general(a, b, (((1,), (1,)), ((), ())), preferred_element_type=F32)


def _pack(v):
    return pltpu.bitcast(v.astype(BF16), U32)


def _unpack(v):
    return pltpu.bitcast(v, BF16)


_LHS = (((0, 1), (3, 1)), ((2, 1), (3, 1)), ((0, 1),), ((3, 1),),
        ((0, 1), (1, 1)), ((2, 1), (0, -1)), ((1, 1), (3, -1)))
_RHS = (((0, 1), (3, 1)), ((0, 1),), ((1, 1), (3, -1)), ((2, 1), (0, -1)),
        ((3, 1),), ((0, 1), (1, 1)), ((2, 1), (3, 1)))
_L2R = (0, 2, 6, 5, 3, 4, 1)
_ORDER = (1, 4, 2, 3, 0, 6, 5)
_OUT_ORDER = (2, 4, 1, 3, 0, 6, 5)
_SWAP = (2, 4, 5, 6)


def _quads(a):
    m, n = a.shape[0] // 2, a.shape[1] // 2
    return a[:m, :n], a[:m, n:], a[m:, :n], a[m:, n:]


def _signed_sum(terms):
    acc = None
    for v, sign in terms:
        acc = v if acc is None else (acc + v if sign > 0 else acc - v)
    return acc


def _operand(tab, quads, i):
    return _signed_sum([(quads[b], sign) for b, sign in tab[i]])


def _operand2(tab, blocks, i, j):
    terms = [(blocks[o][n], so * sn) for o, so in tab[i] for n, sn in tab[j]]
    if len(terms) == 4:
        terms = [terms[0], terms[3], terms[1], terms[2]]
    return _signed_sum(terms)


def _operands_bf16(tab, a):
    q, qf = _quads(a), _quads(a.astype(F32))
    return [q[tab[i][0][0]] if len(tab[i]) == 1 else _operand(tab, qf, i).astype(BF16)
            for i in range(7)]


def _mirror(q):
    return q[1], q[0], q[3], q[2]


def _combine(m):
    m1, m2, m3, m4, m5, m6, m7 = m
    return ((m4 - m5) + m1) + m7, m3 + m5, m2 + m4, ((m3 - m2) + m1) + m6


def _join(c11, c12, c21, c22):
    return jnp.concatenate([jnp.concatenate([c11, c12], axis=1),
                            jnp.concatenate([c21, c22], axis=1)], axis=0)


def _strassen(dot, lhs, rhs):
    m = [None] * 7
    for i in _ORDER:
        m[i] = dot(lhs[i], rhs[i])
    return _combine(m)


def _kernel(x_hbm, wqkv_hbm, wo_hbm, wg_hbm, wu_hbm, wd_hbm, gw_hbm, o_hbm,
            x_v, wq_v, wk_v, wv_v, wo_v, wg_v, wu_v, wd_v, gw_v,
            wqt_v, wq7_v, m_v, k_v, p7_v, z_v, zt_v, kv_v, q0_v, zp_v, g_v, o_v,
            sem, osem):
    S, D = x_v.shape
    F = wg_v.shape[1]
    DH = D // H
    NB = D // LANES
    NP = DH // 2
    HB = LANES // DH
    HD = D // 2
    NC = F // FC

    pairs = []
    for ca, cb in K_STAGES:
        pairs.append((x_hbm.at[pl.ds(0, R1), pl.ds(ca, cb - ca)],
                      x_v.at[pl.ds(0, R1), pl.ds(ca, cb - ca)]))
        pairs.append((wqkv_hbm.at[pl.ds(ca, cb - ca), pl.ds(D, D)], wk_v.at[pl.ds(ca, cb - ca)]))
    n_stage = len(pairs)
    pairs += [
        (gw_hbm, gw_v),
        (wqkv_hbm.at[:, pl.ds(0, D)], wq_v),
        (x_hbm.at[pl.ds(R1, S - R1)], x_v.at[pl.ds(R1, S - R1)]),
        (wqkv_hbm.at[:, pl.ds(2 * D, D)], wv_v),
        (wo_hbm, wo_v),
        (wg_hbm, wg_v),
        (wu_hbm, wu_v),
        (wd_hbm, wd_v),
    ]
    cps = [pltpu.make_async_copy(s, d, sem.at[n]) for n, (s, d) in enumerate(pairs)]
    for c in cps:
        c.start()
    cp_gw, cp_wq, cp_x2, cp_wv, cp_wo, cp_wg, cp_wu, cp_wd = cps[n_stage:]

    def pair_gather(ref, base, n):
        return jnp.concatenate(
            [ref[pl.ds(base + p, n, stride=NP), :] for p in range(NP)], axis=0)

    def x_operands(row):
        return _operands_bf16(_LHS, x_v[pl.ds(row, TS), :])

    def store_gate(t):
        gw = gw_v[...].astype(F32).reshape(1, D)
        xf = x_v[t * TS:(t + 1) * TS, :].astype(F32)
        g = _sigmoid(jnp.sum(xf * gw, axis=1, keepdims=True))
        g_v[t * TS:(t + 1) * TS, :] = jnp.broadcast_to(g, (TS, LANES))

    def p_accumulate(k4, xs, first):
        p11, p12, p21, p22 = [_phi(v) for v in k4]
        colsum = lambda v: jnp.sum(v.reshape(HS // 8, 8, HD), axis=0)
        zz = jnp.concatenate([colsum(p21) + colsum(p11), colsum(p12) + colsum(p22)], axis=1)
        z_v[...] = zz if first else z_v[...] + zz
        blocks = (p11, p21, p12, p22)
        order = (2, 4, 5, 1, 0, 6, 3)
        lhs = {i: _operand(_LHS, blocks, i).astype(BF16).T for i in order}
        for i in order:
            pp = _dot(lhs[i], xs[_L2R[i]])
            p7_v[i] = pp if first else p7_v[i] + pp

    def phase1():
        for n, (ca, cb) in enumerate(K_STAGES):
            cps[2 * n].wait()
            cps[2 * n + 1].wait()
            ks = []
            for a in range(0, R1, TS):
                k = _dot(x_v[a:a + TS, ca:cb], wk_v[ca:cb, :])
                if ca > 0:
                    k = k_v[a:a + TS, :] + k
                if cb < D:
                    k_v[a:a + TS, :] = k
                else:
                    ks.append(k)
            for t, k in enumerate(ks):
                p_accumulate(_quads(k), x_operands(t * TS), t == 0)

        cp_gw.wait()
        cp_wq.wait()
        cp_x2.wait()
        cp_wv.wait()
        cp_wo.wait()

        wqt = pltpu.bitcast(wq_v[...].T, U32)
        for j in range(NB):
            wqt_v[j, 0:HD, :] = wqt[:, j * LANES:(j + 1) * LANES]
        wqp = jnp.concatenate([pair_gather(wqt_v.at[j], 0, H) for j in range(NB)], axis=1)
        w11, w21, w12, w22 = _quads(_unpack(wqp).astype(F32))
        for i in range(7):
            wq7_v[i] = _pack(_operand(_RHS, (w11, w12, w21, w22), i))

        wk7 = _operands_bf16(_RHS, wk_v[...])
        store_gate(2)
        x2 = x_operands(2 * TS)
        k2 = _strassen(_dot, x2, wk7)
        store_gate(3)
        x3 = x_operands(3 * TS)
        k3 = _strassen(_dot, x3, wk7)

        p_accumulate(k2, x2, False)
        q0_v[TS:2 * TS, :] = _join(*_strassen(_dot_nt, x2, [_unpack(wq7_v[i]) for i in range(7)]))
        p_accumulate(k3, x3, False)

        z = jnp.sum(z_v[...], axis=0, keepdims=True)
        zhi = z.astype(BF16).astype(F32)
        rid = lax.broadcasted_iota(jnp.int32, (LANES, D), 0)
        zz = jnp.where(rid == 0, zhi, jnp.where(rid == 1, z - zhi, 0.0)).astype(BF16)
        zt_v[0:HD, :] = pltpu.bitcast(zz.T, U32)
        zp = _unpack(pair_gather(zt_v, 0, H)).T.astype(F32)
        zp_v[...] = jnp.broadcast_to(zp[0:1, :] + zp[1:2, :], (8, D))

        store_gate(0)
        store_gate(1)
        x0, mq = x_operands(0), [None] * 7
        for i in _ORDER[:3]:
            mq[i] = _dot_nt(x0[i], _unpack(wq7_v[i]))
        same_head = (lax.broadcasted_iota(jnp.int32, (LANES, LANES), 0) // DH
                     == lax.broadcasted_iota(jnp.int32, (LANES, LANES), 1) // DH)
        pm = _join(*_combine([p7_v[i] for i in range(7)]))
        for j in range(NB):
            sl = slice(j * LANES, (j + 1) * LANES)
            kv = _dot(pm[sl, :].astype(BF16), wv_v[:, sl])
            kv_v[j * 64:(j + 1) * 64, :] = _pack(jnp.where(same_head, kv, 0.0))
        for i in _ORDER[3:]:
            mq[i] = _dot_nt(x0[i], _unpack(wq7_v[i]))
        q0_v[0:TS, :] = _join(*_combine(mq))
        for j in range(NB):
            kvp = _unpack(pair_gather(kv_v, j * 64, HB))
            mj = _dot(kvp, wo_v[j * LANES:(j + 1) * LANES, :])
            for p in range(NP):
                dst = p * 2 * H + j * 2 * HB
                m_v[dst:dst + 2 * HB, :] = mj[p * 2 * HB:(p + 1) * 2 * HB, :]

        cp_wg.wait()
        cp_wu.wait()
        cp_wd.wait()

    def write_out(row, col, val):
        rows, cols = val.shape
        o_v[pl.ds(row, rows), col:col + cols] = val
        pltpu.make_async_copy(o_v.at[pl.ds(row, rows), pl.ds(col, cols)],
                              o_hbm.at[pl.ds(row, rows), pl.ds(col, cols)], osem).start()

    def gate_up_operands(c):
        left, right = slice(c * FC, c * FC + LANES), slice(c * FC + LANES, (c + 1) * FC)
        top, bot = slice(0, HD), slice(HD, D)
        q = [jnp.concatenate([wg_v[r, s], wu_v[r, s]], axis=1)
             for r, s in ((top, left), (top, right), (bot, left), (bot, right))]
        qf = [v.astype(F32) for v in q]
        return [q[_RHS[i][0][0]] if len(_RHS[i]) == 1 else _operand(_RHS, qf, i).astype(BF16)
                for i in range(7)]

    def attn_weights(q, g):
        pq = _phi(q)
        t = pq * zp_v[0:1, :]
        den = t[:, 0:LANES]
        for j in range(1, NB):
            den = den + t[:, j * LANES:(j + 1) * LANES]
        den = den + pltpu.roll(den, 2 * H, 1)
        even = lax.broadcasted_iota(jnp.int32, den.shape, 1) % 2 == 0
        den = den + jnp.where(even, pltpu.roll(den, LANES - 1, 1), pltpu.roll(den, 1, 1))
        den = den + 1e-6
        inv = pl.reciprocal(den, approx=True)
        inv = inv * (2.0 - den * inv)
        return pq * jnp.concatenate([g * inv] * NB, axis=1)

    def halves_first(v):
        return jnp.concatenate([v[0:HS], v[TS:TS + HS], v[HS:TS], v[TS + HS:T2]], axis=0)

    def body(it, carry):
        pl.when(it == 0)(phase1)
        row = pl.multiple_of(it * T2, T2)
        row1 = pl.multiple_of(row + TS, TS)
        g = g_v[pl.ds(row, T2), :]
        om = halves_first(1.0 - g)
        x1 = x_operands(row1)
        xs = _operands_bf16(_LHS, halves_first(x_v[pl.ds(row, T2), :]))

        hcols = []
        for c in range(NC):
            if c == Q_POS:
                q0 = q0_v[pl.ds(pl.multiple_of(it * TS, TS), TS), :]
                q1 = _join(*_strassen(_dot_nt, x1, [_unpack(wq7_v[i]) for i in range(7)]))
                r = jnp.concatenate([attn_weights(q0, g[0:TS]), attn_weights(q1, g[TS:T2])],
                                    axis=0)
            hs = []
            for n, cb in enumerate(_strassen(_dot, xs, gate_up_operands(c))):
                hg = 0.5 * cb[:, 0:LANES]
                hs.append((hg * (jnp.tanh(hg) + 1.0))
                          * (cb[:, LANES:2 * LANES] * (om[0:TS] if n < 2 else om[TS:T2])))
            hcols.append(halves_first(_join(*hs)))

        groups = [(r, m_v[...])]
        for c in range(0, NC - 1, 2):
            groups.append((jnp.concatenate([hcols[c], hcols[c + 1]], axis=1),
                           wd_v[c * FC:(c + 2) * FC, :].astype(F32)))
        aq = [_quads(a) for a, _ in groups]
        bq = [_quads(b) for _, b in groups]
        a44 = [[_quads(v) for v in q] for q in aq]
        ra, rb = _quads(hcols[NC - 1]), _quads(wd_v[(NC - 1) * FC:NC * FC, :].astype(F32))
        m = [None] * 7
        for i in _OUT_ORDER:
            rest = lambda: _dot(_operand(_LHS, ra, i).astype(BF16),
                                _operand(_RHS, rb, i).astype(BF16))
            flip = _mirror if i in _SWAP else (lambda q: q)
            last = i == _OUT_ORDER[-1]
            if last:
                extra = rest()
            aa = [_quads(_operand(_LHS, q, i)) for q in aq]
            bb = [flip(_quads(_operand(_RHS, q, i))) for q in bq]
            mm = [None] * 7
            for j in _OUT_ORDER:
                for n in range(len(groups)):
                    if n < 2:
                        lhs = _operand2(_LHS, a44[n], i, j)
                        rhs = _operand2(_RHS, [flip(_quads(v)) for v in bq[n]], i, j)
                    else:
                        lhs, rhs = _operand(_LHS, aa[n], j), _operand(_RHS, bb[n], j)
                    d = _dot(lhs.astype(BF16), rhs.astype(BF16))
                    mm[j] = d if mm[j] is None else mm[j] + d
            inner = flip(_combine(mm))
            if not last:
                extra = rest()
            m[i] = _join(*inner) + extra
        c11, c12, c21, c22 = [v.astype(o_v.dtype) for v in _combine(m)]
        write_out(row, HD, c12)
        write_out(row1, 0, c21)
        write_out(row, 0, c11)
        for a in range(0, TS, TAIL_ROWS):
            write_out(pl.multiple_of(row1 + a, TAIL_ROWS), HD, c22[a:a + TAIL_ROWS])
        return carry

    lax.fori_loop(0, S // T2, body, 0)
    pltpu.make_async_copy(o_v, o_hbm, osem).wait()


@jax.jit
def pallas_gated_mix__linear_attn_block__swiglu_ffn__prompt_kernel(
    A_x: jax.Array,
    A_wqkv: jax.Array,
    A_wo: jax.Array,
    B_x: jax.Array,
    B_w_gate: jax.Array,
    B_w_up: jax.Array,
    B_w_down: jax.Array,
    gate_w: jax.Array,
):
    del B_x
    B, S, D = A_x.shape
    F = B_w_gate.shape[1]
    assert B == 1 and S == 2 * T2 and R1 == T2 and D == 4 * LANES and F % (2 * FC) == FC
    hbm = pl.BlockSpec(memory_space=pl.ANY)
    pad = D // 2 + 8
    no_checks = {name: True for name in ("disable_semaphore_checks", "disable_bounds_checks")
                 if hasattr(pltpu.CompilerParams, name)}
    out = pl.pallas_call(
        _kernel,
        out_shape=jax.ShapeDtypeStruct((S, D), A_x.dtype),
        in_specs=[hbm] * 7,
        out_specs=hbm,
        scratch_shapes=[
            pltpu.VMEM((S, D), BF16),
            pltpu.VMEM((D, D), BF16),
            pltpu.VMEM((D, D), BF16),
            pltpu.VMEM((D, D), BF16),
            pltpu.VMEM((D, D), BF16),
            pltpu.VMEM((D, F), BF16),
            pltpu.VMEM((D, F), BF16),
            pltpu.VMEM((F, D), BF16),
            pltpu.VMEM((D,), BF16),
            pltpu.VMEM((D // LANES, pad, LANES), U32),
            pltpu.VMEM((7, D // 4, D // 2), U32),
            pltpu.VMEM((D, D), F32),
            pltpu.VMEM((R1, D), F32),
            pltpu.VMEM((7, D // 2, D // 2), F32),
            pltpu.VMEM((8, D), F32),
            pltpu.VMEM((pad, LANES), U32),
            pltpu.VMEM((pad, LANES), U32),
            pltpu.VMEM((S // T2 * TS, D), F32),
            pltpu.VMEM((8, D), F32),
            pltpu.VMEM((S, LANES), F32),
            pltpu.VMEM((S, D), A_x.dtype),
            pltpu.SemaphoreType.DMA((2 * len(K_STAGES) + 8,)),
            pltpu.SemaphoreType.DMA(()),
        ],
        compiler_params=pltpu.CompilerParams(vmem_limit_bytes=100 * 1024 * 1024, **no_checks),
    )(A_x.reshape(S, D), A_wqkv, A_wo, B_w_gate, B_w_up, B_w_down, gate_w)
    return out.reshape(B, S, D)
```

```python
import jax
import jax.numpy as jnp
from jax import lax
import jax.experimental.pallas as pl
import jax.experimental.pallas.tpu as pltpu

F32 = jnp.float32
BF16 = jnp.bfloat16
U32 = jnp.uint32

H = 32
LANES = 128
TS = 512
HS = TS // 2
T2 = 2 * TS
R1 = 1024
K_STAGES = ((0, 128), (128, 256), (256, 512))
FC = 256
Q_POS = 1
TAIL_ROWS = 32


def _phi(t):
    return jnp.where(t > 0, t + 1.0, jnp.exp(t)) + 1e-6


def _sigmoid(t):
    return 0.5 * jnp.tanh(0.5 * t) + 0.5


def _dot(a, b):
    return jnp.dot(a, b, preferred_element_type=F32)


def _dot_nt(a, b):
    return lax.dot_general(a, b, (((1,), (1,)), ((), ())), preferred_element_type=F32)


def _pack(v):
    return pltpu.bitcast(v.astype(BF16), U32)


def _unpack(v):
    return pltpu.bitcast(v, BF16)


_LHS = (((0, 1), (3, 1)), ((2, 1), (3, 1)), ((0, 1),), ((3, 1),),
        ((0, 1), (1, 1)), ((2, 1), (0, -1)), ((1, 1), (3, -1)))
_RHS = (((0, 1), (3, 1)), ((0, 1),), ((1, 1), (3, -1)), ((2, 1), (0, -1)),
        ((3, 1),), ((0, 1), (1, 1)), ((2, 1), (3, 1)))
_L2R = (0, 2, 6, 5, 3, 4, 1)
_ORDER = (1, 4, 2, 3, 0, 6, 5)
_OUT_ORDER = (2, 4, 1, 3, 0, 6, 5)
_SWAP = (2, 4, 5, 6)


def _quads(a):
    m, n = a.shape[0] // 2, a.shape[1] // 2
    return a[:m, :n], a[:m, n:], a[m:, :n], a[m:, n:]


def _signed_sum(terms):
    acc = None
    for v, sign in terms:
        acc = v if acc is None else (acc + v if sign > 0 else acc - v)
    return acc


def _operand(tab, quads, i):
    return _signed_sum([(quads[b], sign) for b, sign in tab[i]])


def _operand2(tab, blocks, i, j):
    terms = [(blocks[o][n], so * sn) for o, so in tab[i] for n, sn in tab[j]]
    if len(terms) == 4:
        terms = [terms[0], terms[3], terms[1], terms[2]]
    return _signed_sum(terms)


def _operands_bf16(tab, a):
    q, qf = _quads(a), _quads(a.astype(F32))
    return [q[tab[i][0][0]] if len(tab[i]) == 1 else _operand(tab, qf, i).astype(BF16)
            for i in range(7)]


def _mirror(q):
    return q[1], q[0], q[3], q[2]


def _combine(m):
    m1, m2, m3, m4, m5, m6, m7 = m
    return ((m4 - m5) + m1) + m7, m3 + m5, m2 + m4, ((m3 - m2) + m1) + m6


def _join(c11, c12, c21, c22):
    return jnp.concatenate([jnp.concatenate([c11, c12], axis=1),
                            jnp.concatenate([c21, c22], axis=1)], axis=0)


def _strassen(dot, lhs, rhs):
    m = [None] * 7
    for i in _ORDER:
        m[i] = dot(lhs[i], rhs[i])
    return _combine(m)


def _kernel(x_hbm, wqkv_hbm, wo_hbm, wg_hbm, wu_hbm, wd_hbm, gw_hbm, o_hbm,
            x_v, wq_v, wk_v, wv_v, wo_v, wg_v, wu_v, wd_v, gw_v,
            wqt_v, wq7_v, m_v, k_v, pk_v, p7_v, z_v, zt_v, kv_v, q0_v, zp_v, g_v, o_v,
            sem, osem):
    S, D = x_v.shape
    F = wg_v.shape[1]
    DH = D // H
    NB = D // LANES
    NP = DH // 2
    HB = LANES // DH
    HD = D // 2
    NC = F // FC

    pairs = []
    for ca, cb in K_STAGES:
        pairs.append((x_hbm.at[pl.ds(0, R1), pl.ds(ca, cb - ca)],
                      x_v.at[pl.ds(0, R1), pl.ds(ca, cb - ca)]))
        pairs.append((wqkv_hbm.at[pl.ds(ca, cb - ca), pl.ds(D, D)], wk_v.at[pl.ds(ca, cb - ca)]))
    n_stage = len(pairs)
    pairs += [
        (gw_hbm, gw_v),
        (wqkv_hbm.at[:, pl.ds(0, D)], wq_v),
        (x_hbm.at[pl.ds(R1, S - R1)], x_v.at[pl.ds(R1, S - R1)]),
        (wqkv_hbm.at[:, pl.ds(2 * D, D)], wv_v),
        (wo_hbm, wo_v),
        (wg_hbm, wg_v),
        (wu_hbm, wu_v),
        (wd_hbm, wd_v),
    ]
    cps = [pltpu.make_async_copy(s, d, sem.at[n]) for n, (s, d) in enumerate(pairs)]
    for c in cps:
        c.start()
    cp_gw, cp_wq, cp_x2, cp_wv, cp_wo, cp_wg, cp_wu, cp_wd = cps[n_stage:]

    def pair_gather(ref, base, n):
        return jnp.concatenate(
            [ref[pl.ds(base + p, n, stride=NP), :] for p in range(NP)], axis=0)

    def x_operands(row):
        return _operands_bf16(_LHS, x_v[pl.ds(row, TS), :])

    def store_gate(t):
        gw = gw_v[...].astype(F32).reshape(1, D)
        xf = x_v[t * TS:(t + 1) * TS, :].astype(F32)
        g = _sigmoid(jnp.sum(xf * gw, axis=1, keepdims=True))
        g_v[t * TS:(t + 1) * TS, :] = jnp.broadcast_to(g, (TS, LANES))

    def p_accumulate(k4, xs, first, slot=None):
        p11, p12, p21, p22 = [_phi(v) for v in k4]
        colsum = lambda v: jnp.sum(v.reshape(HS // 8, 8, HD), axis=0)
        zz = jnp.concatenate([colsum(p21) + colsum(p11), colsum(p12) + colsum(p22)], axis=1)
        z_v[...] = zz if first else z_v[...] + zz
        blocks = (p11, p21, p12, p22)
        if slot is not None:
            for n, v in enumerate(blocks):
                pk_v[slot, n] = v
            blocks = [pk_v[0, n] for n in range(4)]
        order = (2, 4, 5, 1, 0, 6, 3)
        lhs = {i: _operand(_LHS, blocks, i).astype(BF16).T for i in order}
        for i in order:
            pp = _dot(lhs[i], xs[_L2R[i]])
            p7_v[i] = pp if first else p7_v[i] + pp

    def phase1(it):
        for n, (ca, cb) in enumerate(K_STAGES):
            cps[2 * n].wait()
            cps[2 * n + 1].wait()
            ks = []
            for a in range(0, R1, TS):
                k = _dot(x_v[a:a + TS, ca:cb], wk_v[ca:cb, :])
                if ca > 0:
                    k = k_v[a:a + TS, :] + k
                if cb < D:
                    k_v[a:a + TS, :] = k
                else:
                    ks.append(k)
            for t, k in enumerate(ks):
                p_accumulate(_quads(k), x_operands(t * TS), t == 0)

        cp_gw.wait()
        cp_wq.wait()
        cp_x2.wait()
        cp_wv.wait()
        cp_wo.wait()

        wqt = pltpu.bitcast(wq_v[...].T, U32)
        for j in range(NB):
            wqt_v[j, 0:HD, :] = wqt[:, j * LANES:(j + 1) * LANES]
        wqp = jnp.concatenate([pair_gather(wqt_v.at[j], 0, H) for j in range(NB)], axis=1)
        w11, w21, w12, w22 = _quads(_unpack(wqp).astype(F32))
        for i in range(7):
            wq7_v[i] = _pack(_operand(_RHS, (w11, w12, w21, w22), i))

        wk7 = _operands_bf16(_RHS, wk_v[...])
        store_gate(2)
        x2 = x_operands(2 * TS)
        k2 = _strassen(_dot, x2, wk7)
        store_gate(3)
        x3 = x_operands(3 * TS)
        k3 = _strassen(_dot, x3, wk7)

        p_accumulate(k2, x2, False)
        q0_v[TS:2 * TS, :] = _join(*_strassen(_dot_nt, x2, [_unpack(wq7_v[i]) for i in range(7)]))
        p_accumulate(k3, x3, False, slot=it)

        z = jnp.sum(z_v[...], axis=0, keepdims=True)
        zhi = z.astype(BF16).astype(F32)
        rid = lax.broadcasted_iota(jnp.int32, (LANES, D), 0)
        zz = jnp.where(rid == 0, zhi, jnp.where(rid == 1, z - zhi, 0.0)).astype(BF16)
        zt_v[0:HD, :] = pltpu.bitcast(zz.T, U32)
        zp = _unpack(pair_gather(zt_v, 0, H)).T.astype(F32)
        zp_v[...] = jnp.broadcast_to(zp[0:1, :] + zp[1:2, :], (8, D))

        store_gate(0)
        store_gate(1)
        x0, mq = x_operands(0), [None] * 7
        for i in _ORDER[:3]:
            mq[i] = _dot_nt(x0[i], _unpack(wq7_v[i]))
        same_head = (lax.broadcasted_iota(jnp.int32, (LANES, LANES), 0) // DH
                     == lax.broadcasted_iota(jnp.int32, (LANES, LANES), 1) // DH)
        pm = _join(*_combine([p7_v[i] for i in range(7)]))
        for j in range(NB):
            sl = slice(j * LANES, (j + 1) * LANES)
            kv = _dot(pm[sl, :].astype(BF16), wv_v[:, sl])
            kv_v[j * 64:(j + 1) * 64, :] = _pack(jnp.where(same_head, kv, 0.0))
        for i in _ORDER[3:]:
            mq[i] = _dot_nt(x0[i], _unpack(wq7_v[i]))
        q0_v[0:TS, :] = _join(*_combine(mq))
        for j in range(NB):
            kvp = _unpack(pair_gather(kv_v, j * 64, HB))
            mj = _dot(kvp, wo_v[j * LANES:(j + 1) * LANES, :])
            for p in range(NP):
                dst = p * 2 * H + j * 2 * HB
                m_v[dst:dst + 2 * HB, :] = mj[p * 2 * HB:(p + 1) * 2 * HB, :]

        cp_wg.wait()
        cp_wu.wait()
        cp_wd.wait()

    def write_out(row, col, val):
        rows, cols = val.shape
        o_v[pl.ds(row, rows), col:col + cols] = val
        pltpu.make_async_copy(o_v.at[pl.ds(row, rows), pl.ds(col, cols)],
                              o_hbm.at[pl.ds(row, rows), pl.ds(col, cols)], osem).start()

    def gate_up_operands(c):
        left, right = slice(c * FC, c * FC + LANES), slice(c * FC + LANES, (c + 1) * FC)
        top, bot = slice(0, HD), slice(HD, D)
        q = [jnp.concatenate([wg_v[r, s], wu_v[r, s]], axis=1)
             for r, s in ((top, left), (top, right), (bot, left), (bot, right))]
        qf = [v.astype(F32) for v in q]
        return [q[_RHS[i][0][0]] if len(_RHS[i]) == 1 else _operand(_RHS, qf, i).astype(BF16)
                for i in range(7)]

    def attn_weights(q, g):
        pq = _phi(q)
        t = pq * zp_v[0:1, :]
        den = t[:, 0:LANES]
        for j in range(1, NB):
            den = den + t[:, j * LANES:(j + 1) * LANES]
        den = den + pltpu.roll(den, 2 * H, 1)
        even = lax.broadcasted_iota(jnp.int32, den.shape, 1) % 2 == 0
        den = den + jnp.where(even, pltpu.roll(den, LANES - 1, 1), pltpu.roll(den, 1, 1))
        den = den + 1e-6
        inv = pl.reciprocal(den, approx=True)
        inv = inv * (2.0 - den * inv)
        return pq * jnp.concatenate([g * inv] * NB, axis=1)

    def halves_first(v):
        return jnp.concatenate([v[0:HS], v[TS:TS + HS], v[HS:TS], v[TS + HS:T2]], axis=0)

    def body(it, carry):
        pl.when(it == 0)(lambda: phase1(it))
        row = pl.multiple_of(it * T2, T2)
        row1 = pl.multiple_of(row + TS, TS)
        g = g_v[pl.ds(row, T2), :]
        om = halves_first(1.0 - g)
        x1 = x_operands(row1)
        xs = _operands_bf16(_LHS, halves_first(x_v[pl.ds(row, T2), :]))

        hcols = []
        for c in range(NC):
            if c == Q_POS:
                q0 = q0_v[pl.ds(pl.multiple_of(it * TS, TS), TS), :]
                q1 = _join(*_strassen(_dot_nt, x1, [_unpack(wq7_v[i]) for i in range(7)]))
                r = jnp.concatenate([attn_weights(q0, g[0:TS]), attn_weights(q1, g[TS:T2])],
                                    axis=0)
            hs = []
            for n, cb in enumerate(_strassen(_dot, xs, gate_up_operands(c))):
                hg = 0.5 * cb[:, 0:LANES]
                hs.append((hg * (jnp.tanh(hg) + 1.0))
                          * (cb[:, LANES:2 * LANES] * (om[0:TS] if n < 2 else om[TS:T2])))
            hcols.append(halves_first(_join(*hs)))

        groups = [(r, m_v[...])]
        for c in range(0, NC - 1, 2):
            groups.append((jnp.concatenate([hcols[c], hcols[c + 1]], axis=1),
                           wd_v[c * FC:(c + 2) * FC, :].astype(F32)))
        aq = [_quads(a) for a, _ in groups]
        bq = [_quads(b) for _, b in groups]
        a44 = [[_quads(v) for v in q] for q in aq]
        ra, rb = _quads(hcols[NC - 1]), _quads(wd_v[(NC - 1) * FC:NC * FC, :].astype(F32))
        m = [None] * 7
        for i in _OUT_ORDER:
            rest = lambda: _dot(_operand(_LHS, ra, i).astype(BF16),
                                _operand(_RHS, rb, i).astype(BF16))
            flip = _mirror if i in _SWAP else (lambda q: q)
            last = i == _OUT_ORDER[-1]
            if last:
                extra = rest()
            aa = [_quads(_operand(_LHS, q, i)) for q in aq]
            bb = [flip(_quads(_operand(_RHS, q, i))) for q in bq]
            mm = [None] * 7
            for j in _OUT_ORDER:
                for n in range(len(groups)):
                    if n in (0, 3):
                        lhs = _operand2(_LHS, a44[n], i, j)
                        rhs = _operand2(_RHS, [flip(_quads(v)) for v in bq[n]], i, j)
                    else:
                        lhs, rhs = _operand(_LHS, aa[n], j), _operand(_RHS, bb[n], j)
                    d = _dot(lhs.astype(BF16), rhs.astype(BF16))
                    mm[j] = d if mm[j] is None else mm[j] + d
            inner = flip(_combine(mm))
            if not last:
                extra = rest()
            m[i] = _join(*inner) + extra
        c11, c12, c21, c22 = [v.astype(o_v.dtype) for v in _combine(m)]
        write_out(row, HD, c12)
        write_out(row1, 0, c21)
        write_out(row, 0, c11)
        for a in range(0, TS, TAIL_ROWS):
            write_out(pl.multiple_of(row1 + a, TAIL_ROWS), HD, c22[a:a + TAIL_ROWS])
        return carry

    lax.fori_loop(0, S // T2, body, 0)
    pltpu.make_async_copy(o_v, o_hbm, osem).wait()


@jax.jit
def pallas_gated_mix__linear_attn_block__swiglu_ffn__prompt_kernel(
    A_x: jax.Array,
    A_wqkv: jax.Array,
    A_wo: jax.Array,
    B_x: jax.Array,
    B_w_gate: jax.Array,
    B_w_up: jax.Array,
    B_w_down: jax.Array,
    gate_w: jax.Array,
):
    del B_x
    B, S, D = A_x.shape
    F = B_w_gate.shape[1]
    assert B == 1 and S == 2 * T2 and R1 == T2 and D == 4 * LANES and F % (2 * FC) == FC
    hbm = pl.BlockSpec(memory_space=pl.ANY)
    pad = D // 2 + 8
    no_checks = {name: True for name in ("disable_semaphore_checks", "disable_bounds_checks")
                 if hasattr(pltpu.CompilerParams, name)}
    out = pl.pallas_call(
        _kernel,
        out_shape=jax.ShapeDtypeStruct((S, D), A_x.dtype),
        in_specs=[hbm] * 7,
        out_specs=hbm,
        scratch_shapes=[
            pltpu.VMEM((S, D), BF16),
            pltpu.VMEM((D, D), BF16),
            pltpu.VMEM((D, D), BF16),
            pltpu.VMEM((D, D), BF16),
            pltpu.VMEM((D, D), BF16),
            pltpu.VMEM((D, F), BF16),
            pltpu.VMEM((D, F), BF16),
            pltpu.VMEM((F, D), BF16),
            pltpu.VMEM((D,), BF16),
            pltpu.VMEM((D // LANES, pad, LANES), U32),
            pltpu.VMEM((7, D // 4, D // 2), U32),
            pltpu.VMEM((D, D), F32),
            pltpu.VMEM((R1, D), F32),
            pltpu.VMEM((S // T2, 4, HS, D // 2), F32),
            pltpu.VMEM((7, D // 2, D // 2), F32),
            pltpu.VMEM((8, D), F32),
            pltpu.VMEM((pad, LANES), U32),
            pltpu.VMEM((pad, LANES), U32),
            pltpu.VMEM((S // T2 * TS, D), F32),
            pltpu.VMEM((8, D), F32),
            pltpu.VMEM((S, LANES), F32),
            pltpu.VMEM((S, D), A_x.dtype),
            pltpu.SemaphoreType.DMA((2 * len(K_STAGES) + 8,)),
            pltpu.SemaphoreType.DMA(()),
        ],
        compiler_params=pltpu.CompilerParams(vmem_limit_bytes=100 * 1024 * 1024, **no_checks),
    )(A_x.reshape(S, D), A_wqkv, A_wo, B_w_gate, B_w_up, B_w_down, gate_w)
    return out.reshape(B, S, D)
```

```python
import jax
import jax.numpy as jnp
from jax import lax
import jax.experimental.pallas as pl
import jax.experimental.pallas.tpu as pltpu

F32 = jnp.float32
BF16 = jnp.bfloat16
U32 = jnp.uint32

H = 32
LANES = 128
TS = 512
HS = TS // 2
T2 = 2 * TS
R1 = 1024
K_STAGES = ((0, 128), (128, 256), (256, 512))
FC = 256
TAIL_ROWS = 32


def _phi(t):
    return jnp.where(t > 0, t + 1.0, jnp.exp(t)) + 1e-6


def _sigmoid(t):
    return 0.5 * jnp.tanh(0.5 * t) + 0.5


def _dot(a, b):
    return jnp.dot(a, b, preferred_element_type=F32)


def _dot_nt(a, b):
    return lax.dot_general(a, b, (((1,), (1,)), ((), ())), preferred_element_type=F32)


def _pack(v):
    return pltpu.bitcast(v.astype(BF16), U32)


def _unpack(v):
    return pltpu.bitcast(v, BF16)


_LHS = (((0, 1), (3, 1)), ((2, 1), (3, 1)), ((0, 1),), ((3, 1),),
        ((0, 1), (1, 1)), ((2, 1), (0, -1)), ((1, 1), (3, -1)))
_RHS = (((0, 1), (3, 1)), ((0, 1),), ((1, 1), (3, -1)), ((2, 1), (0, -1)),
        ((3, 1),), ((0, 1), (1, 1)), ((2, 1), (3, 1)))
_L2R = (0, 2, 6, 5, 3, 4, 1)
_ORDER = (1, 4, 2, 3, 0, 6, 5)
_OUT_ORDER = (2, 4, 1, 3, 0, 6, 5)
_SWAP = (2, 4, 5, 6)


def _quads(a):
    m, n = a.shape[0] // 2, a.shape[1] // 2
    return a[:m, :n], a[:m, n:], a[m:, :n], a[m:, n:]


def _signed_sum(terms):
    acc = None
    for v, sign in terms:
        acc = v if acc is None else (acc + v if sign > 0 else acc - v)
    return acc


def _operand(tab, quads, i):
    return _signed_sum([(quads[b], sign) for b, sign in tab[i]])


def _operand2(tab, blocks, i, j):
    terms = [(blocks[o][n], so * sn) for o, so in tab[i] for n, sn in tab[j]]
    if len(terms) == 4:
        terms = [terms[0], terms[3], terms[1], terms[2]]
    return _signed_sum(terms)


def _operands_bf16(tab, a):
    q, qf = _quads(a), _quads(a.astype(F32))
    return [q[tab[i][0][0]] if len(tab[i]) == 1 else _operand(tab, qf, i).astype(BF16)
            for i in range(7)]


def _mirror(q):
    return q[1], q[0], q[3], q[2]


def _combine(m):
    m1, m2, m3, m4, m5, m6, m7 = m
    return ((m4 - m5) + m1) + m7, m3 + m5, m2 + m4, ((m3 - m2) + m1) + m6


def _join(c11, c12, c21, c22):
    return jnp.concatenate([jnp.concatenate([c11, c12], axis=1),
                            jnp.concatenate([c21, c22], axis=1)], axis=0)


def _strassen(dot, lhs, rhs):
    m = [None] * 7
    for i in _ORDER:
        m[i] = dot(lhs[i], rhs[i])
    return _combine(m)


_LAM = (-1.5, -0.5, 0.5, 1.5)
_PAIRS = ((0, 1), (0, 2), (1, 2), (0, 3), (1, 3), (2, 3))


def _times(c, v):
    return v if c == 1.0 else c * v


def _kernel(x_hbm, wqkv_hbm, wo_hbm, wg_hbm, wu_hbm, wd_hbm, gw_hbm, o_hbm,
            x_v, wq_v, wk_v, wv_v, wo_v, wg_v, wu_v, wd_v, gw_v,
            wqt_v, wq7_v, m_v, k_v, pk_v, p7_v, z_v, zt_v, kv_v, q0_v, zp_v, g_v, o_v,
            sem, osem):
    S, D = x_v.shape
    F = wg_v.shape[1]
    DH = D // H
    NB = D // LANES
    NP = DH // 2
    HB = LANES // DH
    HD = D // 2
    NC = F // FC

    pairs = []
    for ca, cb in K_STAGES:
        pairs.append((x_hbm.at[pl.ds(0, R1), pl.ds(ca, cb - ca)],
                      x_v.at[pl.ds(0, R1), pl.ds(ca, cb - ca)]))
        pairs.append((wqkv_hbm.at[pl.ds(ca, cb - ca), pl.ds(D, D)], wk_v.at[pl.ds(ca, cb - ca)]))
    n_stage = len(pairs)
    pairs += [
        (gw_hbm, gw_v),
        (wqkv_hbm.at[:, pl.ds(0, D)], wq_v),
        (x_hbm.at[pl.ds(R1, S - R1)], x_v.at[pl.ds(R1, S - R1)]),
        (wqkv_hbm.at[:, pl.ds(2 * D, D)], wv_v),
        (wo_hbm, wo_v),
        (wg_hbm, wg_v),
        (wu_hbm, wu_v),
        (wd_hbm, wd_v),
    ]
    cps = [pltpu.make_async_copy(s, d, sem.at[n]) for n, (s, d) in enumerate(pairs)]
    for c in cps:
        c.start()
    cp_gw, cp_wq, cp_x2, cp_wv, cp_wo, cp_wg, cp_wu, cp_wd = cps[n_stage:]

    def pair_gather(ref, base, n):
        return jnp.concatenate(
            [ref[pl.ds(base + p, n, stride=NP), :] for p in range(NP)], axis=0)

    def x_operands(row):
        return _operands_bf16(_LHS, x_v[pl.ds(row, TS), :])

    def store_gate(t):
        gw = gw_v[...].astype(F32).reshape(1, D)
        xf = x_v[t * TS:(t + 1) * TS, :].astype(F32)
        g = _sigmoid(jnp.sum(xf * gw, axis=1, keepdims=True))
        g_v[t * TS:(t + 1) * TS, :] = jnp.broadcast_to(g, (TS, LANES))

    def p_accumulate(k4, xs, first, slot=None):
        p11, p12, p21, p22 = [_phi(v) for v in k4]
        colsum = lambda v: jnp.sum(v.reshape(HS // 8, 8, HD), axis=0)
        zz = jnp.concatenate([colsum(p21) + colsum(p11), colsum(p12) + colsum(p22)], axis=1)
        z_v[...] = zz if first else z_v[...] + zz
        blocks = (p11, p21, p12, p22)
        if slot is not None:
            for n, v in enumerate(blocks):
                pk_v[slot, n] = v
            blocks = [pk_v[0, n] for n in range(4)]
        order = (2, 4, 5, 1, 0, 6, 3)
        lhs = {i: _operand(_LHS, blocks, i).astype(BF16).T for i in order}
        for i in order:
            pp = _dot(lhs[i], xs[_L2R[i]])
            p7_v[i] = pp if first else p7_v[i] + pp

    def phase1(it):
        for n, (ca, cb) in enumerate(K_STAGES):
            cps[2 * n].wait()
            cps[2 * n + 1].wait()
            ks = []
            for a in range(0, R1, TS):
                k = _dot(x_v[a:a + TS, ca:cb], wk_v[ca:cb, :])
                if ca > 0:
                    k = k_v[a:a + TS, :] + k
                if cb < D:
                    k_v[a:a + TS, :] = k
                else:
                    ks.append(k)
            for t, k in enumerate(ks):
                p_accumulate(_quads(k), x_operands(t * TS), t == 0)

        cp_gw.wait()
        cp_wq.wait()
        cp_x2.wait()
        cp_wv.wait()
        cp_wo.wait()

        wqt = pltpu.bitcast(wq_v[...].T, U32)
        for j in range(NB):
            wqt_v[j, 0:HD, :] = wqt[:, j * LANES:(j + 1) * LANES]
        wqp = jnp.concatenate([pair_gather(wqt_v.at[j], 0, H) for j in range(NB)], axis=1)
        w11, w21, w12, w22 = _quads(_unpack(wqp).astype(F32))
        for i in range(7):
            wq7_v[i] = _pack(_operand(_RHS, (w11, w12, w21, w22), i))

        wk7 = _operands_bf16(_RHS, wk_v[...])
        store_gate(2)
        x2 = x_operands(2 * TS)
        k2 = _strassen(_dot, x2, wk7)
        store_gate(3)
        x3 = x_operands(3 * TS)
        k3 = _strassen(_dot, x3, wk7)

        p_accumulate(k2, x2, False)
        q0_v[TS:2 * TS, :] = _join(*_strassen(_dot_nt, x2, [_unpack(wq7_v[i]) for i in range(7)]))
        p_accumulate(k3, x3, False, slot=it)

        z = jnp.sum(z_v[...], axis=0, keepdims=True)
        zhi = z.astype(BF16).astype(F32)
        rid = lax.broadcasted_iota(jnp.int32, (LANES, D), 0)
        zz = jnp.where(rid == 0, zhi, jnp.where(rid == 1, z - zhi, 0.0)).astype(BF16)
        zt_v[0:HD, :] = pltpu.bitcast(zz.T, U32)
        zp = _unpack(pair_gather(zt_v, 0, H)).T.astype(F32)
        zp_v[...] = jnp.broadcast_to(zp[0:1, :] + zp[1:2, :], (8, D))

        store_gate(0)
        store_gate(1)
        x0, mq = x_operands(0), [None] * 7
        for i in _ORDER[:3]:
            mq[i] = _dot_nt(x0[i], _unpack(wq7_v[i]))
        same_head = (lax.broadcasted_iota(jnp.int32, (LANES, LANES), 0) // DH
                     == lax.broadcasted_iota(jnp.int32, (LANES, LANES), 1) // DH)
        pm = _join(*_combine([p7_v[i] for i in range(7)]))
        for j in range(NB):
            sl = slice(j * LANES, (j + 1) * LANES)
            kv = _dot(pm[sl, :].astype(BF16), wv_v[:, sl])
            kv_v[j * 64:(j + 1) * 64, :] = _pack(jnp.where(same_head, kv, 0.0))
        for i in _ORDER[3:]:
            mq[i] = _dot_nt(x0[i], _unpack(wq7_v[i]))
        q0_v[0:TS, :] = _join(*_combine(mq))
        for j in range(NB):
            kvp = _unpack(pair_gather(kv_v, j * 64, HB))
            mj = _dot(kvp, wo_v[j * LANES:(j + 1) * LANES, :])
            for p in range(NP):
                dst = p * 2 * H + j * 2 * HB
                m_v[dst:dst + 2 * HB, :] = mj[p * 2 * HB:(p + 1) * 2 * HB, :]

        cp_wg.wait()
        cp_wu.wait()
        cp_wd.wait()

    def write_out(row, col, val):
        rows, cols = val.shape
        o_v[pl.ds(row, rows), col:col + cols] = val
        pltpu.make_async_copy(o_v.at[pl.ds(row, rows), pl.ds(col, cols)],
                              o_hbm.at[pl.ds(row, rows), pl.ds(col, cols)], osem).start()

    def attn_weights(q, g):
        pq = _phi(q)
        t = pq * zp_v[0:1, :]
        den = t[:, 0:LANES]
        for j in range(1, NB):
            den = den + t[:, j * LANES:(j + 1) * LANES]
        den = den + pltpu.roll(den, 2 * H, 1)
        even = lax.broadcasted_iota(jnp.int32, den.shape, 1) % 2 == 0
        den = den + jnp.where(even, pltpu.roll(den, LANES - 1, 1), pltpu.roll(den, 1, 1))
        den = den + 1e-6
        inv = pl.reciprocal(den, approx=True)
        inv = inv * (2.0 - den * inv)
        return pq * jnp.concatenate([g * inv] * NB, axis=1)

    def body(it, carry):
        pl.when(it == 0)(lambda: phase1(it))
        row = pl.multiple_of(it * T2, T2)
        row1 = pl.multiple_of(row + TS, TS)
        g = g_v[pl.ds(row, T2), :]
        omg = 1.0 - g
        x1 = x_operands(row1)

        xt = x_v[pl.ds(row, T2), :]
        xf = xt.astype(F32)
        rows = [slice(i * HS, (i + 1) * HS) for i in range(4)]
        a1b = [xt[r, 0:HD] for r in rows]
        a1 = [xf[r, 0:HD] for r in rows]
        y = [_LAM[i] * a1[i] + xf[rows[i], HD:D] for i in range(4)]
        yb = [v.astype(BF16) for v in y]
        mixed = {}

        def mixed_lhs(i, j):
            if (i, j) not in mixed:
                e = _times(1.0 / (_LAM[j] - _LAM[i]), y[j] - y[i])
                mixed[i, j] = [v.astype(BF16) for v in (e, a1[j] - e, a1[i] - e)]
            return mixed[i, j]

        hb = {}

        def activate(i, col, c):
            hg = 0.5 * c[:, 0:LANES]
            hb[i, col] = (hg * (jnp.tanh(hg) + 1.0)) * (c[:, LANES:2 * LANES] * omg[rows[i]])

        def gate_up(cols, pairs):
            b2b, b2, u, dd, ee = {}, {}, {}, {}, {}
            for i, col in cols.items():
                cs = slice(col * LANES, (col + 1) * LANES)
                b1 = jnp.concatenate([wg_v[0:HD, cs], wu_v[0:HD, cs]], axis=1).astype(F32)
                b2b[i] = jnp.concatenate([wg_v[HD:D, cs], wu_v[HD:D, cs]], axis=1)
                b2[i] = b2b[i].astype(F32)
                u[i] = b1 - _LAM[i] * b2[i]
            for i, j in pairs:
                for n in (i, j):
                    if n not in dd:
                        ee[n] = _dot(yb[n], b2b[n])
                        dd[n] = _dot(a1b[n], u[n].astype(BF16))
                        activate(n, cols[n], dd[n] + ee[n])
                d = _LAM[j] - _LAM[i]
                l0, lj, li = mixed_lhs(i, j)
                uu = u[i] + u[j]
                m0 = _dot(l0, uu.astype(BF16))
                mj = _dot(lj, (uu - _times(d, b2[i])).astype(BF16))
                mi = _dot(li, (uu + _times(d, b2[j])).astype(BF16))
                activate(j, cols[i], ((ee[i] - dd[j]) + m0) + mj)
                activate(i, cols[j], ((ee[j] - dd[i]) + m0) + mi)

        n_blk = F // LANES
        for c0 in range(0, n_blk - 2, 4):
            gate_up({i: c0 + i for i in range(4)}, _PAIRS)
            if c0 == 0:
                q0 = q0_v[pl.ds(pl.multiple_of(it * TS, TS), TS), :]
                q1 = _join(*_strassen(_dot_nt, x1, [_unpack(wq7_v[i]) for i in range(7)]))
                r = jnp.concatenate([attn_weights(q0, g[0:TS]), attn_weights(q1, g[TS:T2])],
                                    axis=0)
        gate_up({1: n_blk - 2, 2: n_blk - 1}, ((1, 2),))
        gate_up({0: n_blk - 2, 3: n_blk - 1}, ((0, 3),))
        hcols = [jnp.concatenate([jnp.concatenate([hb[i, 2 * c], hb[i, 2 * c + 1]], axis=1)
                                  for i in range(4)], axis=0) for c in range(NC)]

        groups = [(r, m_v[...])]
        for c in range(0, NC - 1, 2):
            groups.append((jnp.concatenate([hcols[c], hcols[c + 1]], axis=1),
                           wd_v[c * FC:(c + 2) * FC, :].astype(F32)))
        aq = [_quads(a) for a, _ in groups]
        bq = [_quads(b) for _, b in groups]
        a44 = [[_quads(v) for v in q] for q in aq]
        ra, rb = _quads(hcols[NC - 1]), _quads(wd_v[(NC - 1) * FC:NC * FC, :].astype(F32))
        m = [None] * 7
        for i in _OUT_ORDER:
            rest = lambda: _dot(_operand(_LHS, ra, i).astype(BF16),
                                _operand(_RHS, rb, i).astype(BF16))
            flip = _mirror if i in _SWAP else (lambda q: q)
            last = i == _OUT_ORDER[-1]
            if last:
                extra = rest()
            aa = [_quads(_operand(_LHS, q, i)) for q in aq]
            bb = [flip(_quads(_operand(_RHS, q, i))) for q in bq]
            mm = [None] * 7
            for j in _OUT_ORDER:
                for n in range(len(groups)):
                    if n in (0, 3):
                        lhs = _operand2(_LHS, a44[n], i, j)
                        rhs = _operand2(_RHS, [flip(_quads(v)) for v in bq[n]], i, j)
                    else:
                        lhs, rhs = _operand(_LHS, aa[n], j), _operand(_RHS, bb[n], j)
                    d = _dot(lhs.astype(BF16), rhs.astype(BF16))
                    mm[j] = d if mm[j] is None else mm[j] + d
            inner = flip(_combine(mm))
            if not last:
                extra = rest()
            m[i] = _join(*inner) + extra
        c11, c12, c21, c22 = [v.astype(o_v.dtype) for v in _combine(m)]
        write_out(row, HD, c12)
        write_out(row1, 0, c21)
        write_out(row, 0, c11)
        for a in range(0, TS, TAIL_ROWS):
            write_out(pl.multiple_of(row1 + a, TAIL_ROWS), HD, c22[a:a + TAIL_ROWS])
        return carry

    lax.fori_loop(0, S // T2, body, 0)
    pltpu.make_async_copy(o_v, o_hbm, osem).wait()


@jax.jit
def pallas_gated_mix__linear_attn_block__swiglu_ffn__prompt_kernel(
    A_x: jax.Array,
    A_wqkv: jax.Array,
    A_wo: jax.Array,
    B_x: jax.Array,
    B_w_gate: jax.Array,
    B_w_up: jax.Array,
    B_w_down: jax.Array,
    gate_w: jax.Array,
):
    del B_x
    B, S, D = A_x.shape
    F = B_w_gate.shape[1]
    assert B == 1 and S == 2 * T2 and R1 == T2 and D == 4 * LANES and F % (2 * FC) == FC
    hbm = pl.BlockSpec(memory_space=pl.ANY)
    pad = D // 2 + 8
    no_checks = {name: True for name in ("disable_semaphore_checks", "disable_bounds_checks")
                 if hasattr(pltpu.CompilerParams, name)}
    out = pl.pallas_call(
        _kernel,
        out_shape=jax.ShapeDtypeStruct((S, D), A_x.dtype),
        in_specs=[hbm] * 7,
        out_specs=hbm,
        scratch_shapes=[
            pltpu.VMEM((S, D), BF16),
            pltpu.VMEM((D, D), BF16),
            pltpu.VMEM((D, D), BF16),
            pltpu.VMEM((D, D), BF16),
            pltpu.VMEM((D, D), BF16),
            pltpu.VMEM((D, F), BF16),
            pltpu.VMEM((D, F), BF16),
            pltpu.VMEM((F, D), BF16),
            pltpu.VMEM((D,), BF16),
            pltpu.VMEM((D // LANES, pad, LANES), U32),
            pltpu.VMEM((7, D // 4, D // 2), U32),
            pltpu.VMEM((D, D), F32),
            pltpu.VMEM((R1, D), F32),
            pltpu.VMEM((S // T2, 4, HS, D // 2), F32),
            pltpu.VMEM((7, D // 2, D // 2), F32),
            pltpu.VMEM((8, D), F32),
            pltpu.VMEM((pad, LANES), U32),
            pltpu.VMEM((pad, LANES), U32),
            pltpu.VMEM((S // T2 * TS, D), F32),
            pltpu.VMEM((8, D), F32),
            pltpu.VMEM((S, LANES), F32),
            pltpu.VMEM((S, D), A_x.dtype),
            pltpu.SemaphoreType.DMA((2 * len(K_STAGES) + 8,)),
            pltpu.SemaphoreType.DMA(()),
        ],
        compiler_params=pltpu.CompilerParams(vmem_limit_bytes=100 * 1024 * 1024, **no_checks),
    )(A_x.reshape(S, D), A_wqkv, A_wo, B_w_gate, B_w_up, B_w_down, gate_w)
    return out.reshape(B, S, D)
```

```python
import jax
import jax.numpy as jnp
from jax import lax
import jax.experimental.pallas as pl
import jax.experimental.pallas.tpu as pltpu

F32 = jnp.float32
BF16 = jnp.bfloat16
U32 = jnp.uint32

H = 32
LANES = 128
TS = 512
HS = TS // 2
T2 = 2 * TS
R1 = 1024
K_STAGES = ((0, 128), (128, 256), (256, 512))
FC = 256
TAIL_ROWS = 32


def _phi(t):
    return jnp.where(t > 0, t + 1.0, jnp.exp(t)) + 1e-6


def _sigmoid(t):
    return 0.5 * jnp.tanh(0.5 * t) + 0.5


def _dot(a, b):
    return jnp.dot(a, b, preferred_element_type=F32)


def _dot_nt(a, b):
    return lax.dot_general(a, b, (((1,), (1,)), ((), ())), preferred_element_type=F32)


def _pack(v):
    return pltpu.bitcast(v.astype(BF16), U32)


def _unpack(v):
    return pltpu.bitcast(v, BF16)


_LHS = (((0, 1), (3, 1)), ((2, 1), (3, 1)), ((0, 1),), ((3, 1),),
        ((0, 1), (1, 1)), ((2, 1), (0, -1)), ((1, 1), (3, -1)))
_RHS = (((0, 1), (3, 1)), ((0, 1),), ((1, 1), (3, -1)), ((2, 1), (0, -1)),
        ((3, 1),), ((0, 1), (1, 1)), ((2, 1), (3, 1)))
_L2R = (0, 2, 6, 5, 3, 4, 1)
_ORDER = (1, 4, 2, 3, 0, 6, 5)
_OUT_ORDER = (2, 4, 1, 3, 0, 6, 5)
_SWAP = (2, 4, 5, 6)


def _quads(a):
    m, n = a.shape[0] // 2, a.shape[1] // 2
    return a[:m, :n], a[:m, n:], a[m:, :n], a[m:, n:]


def _signed_sum(terms):
    acc = None
    for v, sign in terms:
        acc = v if acc is None else (acc + v if sign > 0 else acc - v)
    return acc


def _operand(tab, quads, i):
    return _signed_sum([(quads[b], sign) for b, sign in tab[i]])


def _operand2(tab, blocks, i, j):
    terms = [(blocks[o][n], so * sn) for o, so in tab[i] for n, sn in tab[j]]
    if len(terms) == 4:
        terms = [terms[0], terms[3], terms[1], terms[2]]
    return _signed_sum(terms)


def _operands_bf16(tab, a):
    q, qf = _quads(a), _quads(a.astype(F32))
    return [q[tab[i][0][0]] if len(tab[i]) == 1 else _operand(tab, qf, i).astype(BF16)
            for i in range(7)]


def _mirror(q):
    return q[1], q[0], q[3], q[2]


def _combine(m):
    m1, m2, m3, m4, m5, m6, m7 = m
    return ((m4 - m5) + m1) + m7, m3 + m5, m2 + m4, ((m3 - m2) + m1) + m6


def _join(c11, c12, c21, c22):
    return jnp.concatenate([jnp.concatenate([c11, c12], axis=1),
                            jnp.concatenate([c21, c22], axis=1)], axis=0)


def _strassen(dot, lhs, rhs):
    m = [None] * 7
    for i in _ORDER:
        m[i] = dot(lhs[i], rhs[i])
    return _combine(m)


_LAM = (-1.5, -0.5, 0.5, 1.5)
_PAIRS = ((1, 2), (0, 1), (0, 2), (2, 3), (1, 3), (0, 3))


def _times(c, v):
    return v if c == 1.0 else c * v


def _kernel(x_hbm, wqkv_hbm, wo_hbm, wg_hbm, wu_hbm, wd_hbm, gw_hbm, o_hbm,
            x_v, wq_v, wk_v, wv_v, wo_v, wg_v, wu_v, wd_v, gw_v,
            wqt_v, wq7_v, m_v, k_v, pk_v, p7_v, z_v, zt_v, kv_v, q0_v, zp_v, g_v, o_v,
            sem, osem):
    S, D = x_v.shape
    F = wg_v.shape[1]
    DH = D // H
    NB = D // LANES
    NP = DH // 2
    HB = LANES // DH
    HD = D // 2
    NC = F // FC

    pairs = []
    for ca, cb in K_STAGES:
        pairs.append((x_hbm.at[pl.ds(0, R1), pl.ds(ca, cb - ca)],
                      x_v.at[pl.ds(0, R1), pl.ds(ca, cb - ca)]))
        pairs.append((wqkv_hbm.at[pl.ds(ca, cb - ca), pl.ds(D, D)], wk_v.at[pl.ds(ca, cb - ca)]))
    n_stage = len(pairs)
    pairs += [
        (gw_hbm, gw_v),
        (wqkv_hbm.at[:, pl.ds(0, D)], wq_v),
        (x_hbm.at[pl.ds(R1, S - R1)], x_v.at[pl.ds(R1, S - R1)]),
        (wqkv_hbm.at[:, pl.ds(2 * D, D)], wv_v),
        (wo_hbm, wo_v),
        (wg_hbm, wg_v),
        (wu_hbm, wu_v),
        (wd_hbm, wd_v),
    ]
    cps = [pltpu.make_async_copy(s, d, sem.at[n]) for n, (s, d) in enumerate(pairs)]
    for c in cps:
        c.start()
    cp_gw, cp_wq, cp_x2, cp_wv, cp_wo, cp_wg, cp_wu, cp_wd = cps[n_stage:]

    def pair_gather(ref, base, n):
        return jnp.concatenate(
            [ref[pl.ds(base + p, n, stride=NP), :] for p in range(NP)], axis=0)

    def x_operands(row):
        return _operands_bf16(_LHS, x_v[pl.ds(row, TS), :])

    def store_gate(t):
        gw = gw_v[...].astype(F32).reshape(1, D)
        xf = x_v[t * TS:(t + 1) * TS, :].astype(F32)
        g = _sigmoid(jnp.sum(xf * gw, axis=1, keepdims=True))
        g_v[t * TS:(t + 1) * TS, :] = jnp.broadcast_to(g, (TS, LANES))

    def p_accumulate(k4, xs, first, slot=None):
        p11, p12, p21, p22 = [_phi(v) for v in k4]
        colsum = lambda v: jnp.sum(v.reshape(HS // 8, 8, HD), axis=0)
        zz = jnp.concatenate([colsum(p21) + colsum(p11), colsum(p12) + colsum(p22)], axis=1)
        z_v[...] = zz if first else z_v[...] + zz
        blocks = (p11, p21, p12, p22)
        if slot is not None:
            for n, v in enumerate(blocks):
                pk_v[slot, n] = v
            blocks = [pk_v[0, n] for n in range(4)]
        order = (2, 4, 5, 1, 0, 6, 3)
        lhs = {i: _operand(_LHS, blocks, i).astype(BF16).T for i in order}
        for i in order:
            pp = _dot(lhs[i], xs[_L2R[i]])
            p7_v[i] = pp if first else p7_v[i] + pp

    def phase1(it):
        for n, (ca, cb) in enumerate(K_STAGES):
            cps[2 * n].wait()
            cps[2 * n + 1].wait()
            ks = []
            for a in range(0, R1, TS):
                k = _dot(x_v[a:a + TS, ca:cb], wk_v[ca:cb, :])
                if ca > 0:
                    k = k_v[a:a + TS, :] + k
                if cb < D:
                    k_v[a:a + TS, :] = k
                else:
                    ks.append(k)
            for t, k in enumerate(ks):
                p_accumulate(_quads(k), x_operands(t * TS), t == 0)

        cp_gw.wait()
        cp_wq.wait()
        cp_x2.wait()
        cp_wv.wait()
        cp_wo.wait()

        wqt = pltpu.bitcast(wq_v[...].T, U32)
        for j in range(NB):
            wqt_v[j, 0:HD, :] = wqt[:, j * LANES:(j + 1) * LANES]
        wqp = jnp.concatenate([pair_gather(wqt_v.at[j], 0, H) for j in range(NB)], axis=1)
        w11, w21, w12, w22 = _quads(_unpack(wqp).astype(F32))
        for i in range(7):
            wq7_v[i] = _pack(_operand(_RHS, (w11, w12, w21, w22), i))

        wk7 = _operands_bf16(_RHS, wk_v[...])
        store_gate(2)
        x2 = x_operands(2 * TS)
        k2 = _strassen(_dot, x2, wk7)
        store_gate(3)
        x3 = x_operands(3 * TS)
        k3 = _strassen(_dot, x3, wk7)

        p_accumulate(k2, x2, False)
        q0_v[TS:2 * TS, :] = _join(*_strassen(_dot_nt, x2, [_unpack(wq7_v[i]) for i in range(7)]))
        p_accumulate(k3, x3, False, slot=it)

        z = jnp.sum(z_v[...], axis=0, keepdims=True)
        zhi = z.astype(BF16).astype(F32)
        rid = lax.broadcasted_iota(jnp.int32, (LANES, D), 0)
        zz = jnp.where(rid == 0, zhi, jnp.where(rid == 1, z - zhi, 0.0)).astype(BF16)
        zt_v[0:HD, :] = pltpu.bitcast(zz.T, U32)
        zp = _unpack(pair_gather(zt_v, 0, H)).T.astype(F32)
        zp_v[...] = jnp.broadcast_to(zp[0:1, :] + zp[1:2, :], (8, D))

        store_gate(0)
        store_gate(1)
        x0, mq = x_operands(0), [None] * 7
        for i in _ORDER[:3]:
            mq[i] = _dot_nt(x0[i], _unpack(wq7_v[i]))
        same_head = (lax.broadcasted_iota(jnp.int32, (LANES, LANES), 0) // DH
                     == lax.broadcasted_iota(jnp.int32, (LANES, LANES), 1) // DH)
        pm = _join(*_combine([p7_v[i] for i in range(7)]))
        for j in range(NB):
            sl = slice(j * LANES, (j + 1) * LANES)
            kv = _dot(pm[sl, :].astype(BF16), wv_v[:, sl])
            kv_v[j * 64:(j + 1) * 64, :] = _pack(jnp.where(same_head, kv, 0.0))
        for i in _ORDER[3:]:
            mq[i] = _dot_nt(x0[i], _unpack(wq7_v[i]))
        q0_v[0:TS, :] = _join(*_combine(mq))
        for j in range(NB):
            kvp = _unpack(pair_gather(kv_v, j * 64, HB))
            mj = _dot(kvp, wo_v[j * LANES:(j + 1) * LANES, :])
            for p in range(NP):
                dst = p * 2 * H + j * 2 * HB
                m_v[dst:dst + 2 * HB, :] = mj[p * 2 * HB:(p + 1) * 2 * HB, :]

        cp_wg.wait()
        cp_wu.wait()
        cp_wd.wait()

    def write_out(row, col, val):
        rows, cols = val.shape
        o_v[pl.ds(row, rows), col:col + cols] = val
        pltpu.make_async_copy(o_v.at[pl.ds(row, rows), pl.ds(col, cols)],
                              o_hbm.at[pl.ds(row, rows), pl.ds(col, cols)], osem).start()

    def attn_weights(q, g):
        pq = _phi(q)
        t = pq * zp_v[0:1, :]
        den = t[:, 0:LANES]
        for j in range(1, NB):
            den = den + t[:, j * LANES:(j + 1) * LANES]
        den = den + pltpu.roll(den, 2 * H, 1)
        even = lax.broadcasted_iota(jnp.int32, den.shape, 1) % 2 == 0
        den = den + jnp.where(even, pltpu.roll(den, LANES - 1, 1), pltpu.roll(den, 1, 1))
        den = den + 1e-6
        inv = pl.reciprocal(den, approx=True)
        inv = inv * (2.0 - den * inv)
        return pq * jnp.concatenate([g * inv] * NB, axis=1)

    def body(it, carry):
        pl.when(it == 0)(lambda: phase1(it))
        row = pl.multiple_of(it * T2, T2)
        row1 = pl.multiple_of(row + TS, TS)
        g = g_v[pl.ds(row, T2), :]
        omg = 1.0 - g
        x1 = x_operands(row1)

        xt = x_v[pl.ds(row, T2), :]
        xf = xt.astype(F32)
        rows = [slice(i * HS, (i + 1) * HS) for i in range(4)]
        a1b = [xt[r, 0:HD] for r in rows]
        a1 = [xf[r, 0:HD] for r in rows]
        y = [_LAM[i] * a1[i] + xf[rows[i], HD:D] for i in range(4)]
        yb = [v.astype(BF16) for v in y]
        mixed = {}

        def mixed_lhs(i, j):
            if (i, j) not in mixed:
                e = _times(1.0 / (_LAM[j] - _LAM[i]), y[j] - y[i])
                mixed[i, j] = [v.astype(BF16) for v in (e, a1[j] - e, a1[i] - e)]
            return mixed[i, j]

        hb = {}

        def activate(i, col, c):
            hg = 0.5 * c[:, 0:LANES]
            hb[i, col] = (hg * (jnp.tanh(hg) + 1.0)) * (c[:, LANES:2 * LANES] * omg[rows[i]])

        def gate_up(cols, pairs):
            b2b, b2, ub, u, dd, ee = {}, {}, {}, {}, {}, {}
            for i, col in cols.items():
                cs = slice(col * LANES, (col + 1) * LANES)
                b1 = jnp.concatenate([wg_v[0:HD, cs], wu_v[0:HD, cs]], axis=1).astype(F32)
                b2b[i] = jnp.concatenate([wg_v[HD:D, cs], wu_v[HD:D, cs]], axis=1)
                b2[i] = b2b[i].astype(F32)
                ub[i] = (b1 - _LAM[i] * b2[i]).astype(BF16)
                u[i] = ub[i].astype(F32)
            for i, j in pairs:
                for n in (i, j):
                    if n not in dd:
                        ee[n] = _dot(yb[n], b2b[n])
                        dd[n] = _dot(a1b[n], ub[n])
                        activate(n, cols[n], dd[n] + ee[n])
                d = _LAM[j] - _LAM[i]
                l0, lj, li = mixed_lhs(i, j)
                uu = u[i] + u[j]
                m0 = _dot(l0, uu.astype(BF16))
                mj = _dot(lj, (uu - _times(d, b2[i])).astype(BF16))
                mi = _dot(li, (uu + _times(d, b2[j])).astype(BF16))
                activate(j, cols[i], ((ee[i] - dd[j]) + m0) + mj)
                activate(i, cols[j], ((ee[j] - dd[i]) + m0) + mi)

        n_blk = F // LANES
        for c0 in range(0, n_blk - 2, 4):
            gate_up({i: c0 + i for i in range(4)}, _PAIRS)
            if c0 == 0:
                q0 = q0_v[pl.ds(pl.multiple_of(it * TS, TS), TS), :]
                q1 = _join(*_strassen(_dot_nt, x1, [_unpack(wq7_v[i]) for i in range(7)]))
                r = jnp.concatenate([attn_weights(q0, g[0:TS]), attn_weights(q1, g[TS:T2])],
                                    axis=0)
        gate_up({1: n_blk - 2, 2: n_blk - 1}, ((1, 2),))
        gate_up({0: n_blk - 2, 3: n_blk - 1}, ((0, 3),))
        hcols = [jnp.concatenate([jnp.concatenate([hb[i, 2 * c], hb[i, 2 * c + 1]], axis=1)
                                  for i in range(4)], axis=0) for c in range(NC)]

        groups = [(r, m_v[...])]
        for c in range(0, NC - 1, 2):
            groups.append((jnp.concatenate([hcols[c], hcols[c + 1]], axis=1),
                           wd_v[c * FC:(c + 2) * FC, :].astype(F32)))
        aq = [_quads(a) for a, _ in groups]
        bq = [_quads(b) for _, b in groups]
        a44 = [[_quads(v) for v in q] for q in aq]
        ra, rb = _quads(hcols[NC - 1]), _quads(wd_v[(NC - 1) * FC:NC * FC, :].astype(F32))
        m = [None] * 7
        for i in _OUT_ORDER:
            rest = lambda: _dot(_operand(_LHS, ra, i).astype(BF16),
                                _operand(_RHS, rb, i).astype(BF16))
            flip = _mirror if i in _SWAP else (lambda q: q)
            last = i == _OUT_ORDER[-1]
            if last:
                extra = rest()
            aa = [_quads(_operand(_LHS, q, i)) for q in aq]
            bb = [flip(_quads(_operand(_RHS, q, i))) for q in bq]
            mm = [None] * 7
            for j in _OUT_ORDER:
                for n in (1, 2, 3, 0):
                    lhs = (_operand2(_LHS, a44[n], i, j) if n in (0, 3)
                           else _operand(_LHS, aa[n], j))
                    rhs = (_operand2(_RHS, [flip(_quads(v)) for v in bq[n]], i, j) if n > 0
                           else _operand(_RHS, bb[n], j))
                    d = _dot(lhs.astype(BF16), rhs.astype(BF16))
                    mm[j] = d if mm[j] is None else mm[j] + d
            inner = flip(_combine(mm))
            if not last:
                extra = rest()
            m[i] = _join(*inner) + extra
        c11, c12, c21, c22 = [v.astype(o_v.dtype) for v in _combine(m)]
        write_out(row, HD, c12)
        write_out(row1, 0, c21)
        write_out(row, 0, c11)
        for a in range(0, TS, TAIL_ROWS):
            write_out(pl.multiple_of(row1 + a, TAIL_ROWS), HD, c22[a:a + TAIL_ROWS])
        return carry

    lax.fori_loop(0, S // T2, body, 0)
    pltpu.make_async_copy(o_v, o_hbm, osem).wait()


@jax.jit
def pallas_gated_mix__linear_attn_block__swiglu_ffn__prompt_kernel(
    A_x: jax.Array,
    A_wqkv: jax.Array,
    A_wo: jax.Array,
    B_x: jax.Array,
    B_w_gate: jax.Array,
    B_w_up: jax.Array,
    B_w_down: jax.Array,
    gate_w: jax.Array,
):
    del B_x
    B, S, D = A_x.shape
    F = B_w_gate.shape[1]
    assert B == 1 and S == 2 * T2 and R1 == T2 and D == 4 * LANES and F % (2 * FC) == FC
    hbm = pl.BlockSpec(memory_space=pl.ANY)
    pad = D // 2 + 8
    no_checks = {name: True for name in ("disable_semaphore_checks", "disable_bounds_checks")
                 if hasattr(pltpu.CompilerParams, name)}
    out = pl.pallas_call(
        _kernel,
        out_shape=jax.ShapeDtypeStruct((S, D), A_x.dtype),
        in_specs=[hbm] * 7,
        out_specs=hbm,
        scratch_shapes=[
            pltpu.VMEM((S, D), BF16),
            pltpu.VMEM((D, D), BF16),
            pltpu.VMEM((D, D), BF16),
            pltpu.VMEM((D, D), BF16),
            pltpu.VMEM((D, D), BF16),
            pltpu.VMEM((D, F), BF16),
            pltpu.VMEM((D, F), BF16),
            pltpu.VMEM((F, D), BF16),
            pltpu.VMEM((D,), BF16),
            pltpu.VMEM((D // LANES, pad, LANES), U32),
            pltpu.VMEM((7, D // 4, D // 2), U32),
            pltpu.VMEM((D, D), F32),
            pltpu.VMEM((R1, D), F32),
            pltpu.VMEM((S // T2, 4, HS, D // 2), F32),
            pltpu.VMEM((7, D // 2, D // 2), F32),
            pltpu.VMEM((8, D), F32),
            pltpu.VMEM((pad, LANES), U32),
            pltpu.VMEM((pad, LANES), U32),
            pltpu.VMEM((S // T2 * TS, D), F32),
            pltpu.VMEM((8, D), F32),
            pltpu.VMEM((S, LANES), F32),
            pltpu.VMEM((S, D), A_x.dtype),
            pltpu.SemaphoreType.DMA((2 * len(K_STAGES) + 8,)),
            pltpu.SemaphoreType.DMA(()),
        ],
        compiler_params=pltpu.CompilerParams(vmem_limit_bytes=100 * 1024 * 1024, **no_checks),
    )(A_x.reshape(S, D), A_wqkv, A_wo, B_w_gate, B_w_up, B_w_down, gate_w)
    return out.reshape(B, S, D)
```

```python
import jax
import jax.numpy as jnp
from jax import lax
import jax.experimental.pallas as pl
import jax.experimental.pallas.tpu as pltpu

F32 = jnp.float32
BF16 = jnp.bfloat16
U32 = jnp.uint32
NT = (((1,), (1,)), ((), ()))

H = 32
LANES = 128
KT = 512
TS = 256
T2 = 1024
R1 = 1024
K_STAGES = ((0, 128), (128, 256), (256, 512))
TAIL_ROWS = 32


def _phi(t):
    return jnp.where(t > 0, t + 1.0, jnp.exp(t)) + 1e-6


def _sigmoid(t):
    return 0.5 * jnp.tanh(0.5 * t) + 0.5


def _dot(a, b):
    return jnp.dot(a, b, preferred_element_type=F32)


def _kernel(x_hbm, wqkv_hbm, wo_hbm, wg_hbm, wu_hbm, wd_hbm, gw_hbm, o_hbm,
            x_v, wq_v, wk_v, wv_v, wo_v, wg_v, wu_v, wd_v, gw_v,
            wqp_v, wqt_v, k_v, p_v, z_v, zt_v, kv_v, m_v, q0_v, zp_v, o_v, sem, osem):
    S, D = x_v.shape
    F = wg_v.shape[1]
    DH = D // H
    NB = D // LANES
    NP = DH // 2
    HB = LANES // DH
    n_iter = S // T2
    n_sub = T2 // TS
    fc = F // 2

    pairs = []
    for ca, cb in K_STAGES:
        pairs.append((x_hbm.at[pl.ds(0, R1), pl.ds(ca, cb - ca)],
                      x_v.at[pl.ds(0, R1), pl.ds(ca, cb - ca)]))
        pairs.append((wqkv_hbm.at[pl.ds(ca, cb - ca), pl.ds(D, D)], wk_v.at[pl.ds(ca, cb - ca)]))
    n_stage = len(pairs)
    pairs += [
        (wqkv_hbm.at[:, pl.ds(0, D)], wq_v),
        (x_hbm.at[pl.ds(R1, S - R1)], x_v.at[pl.ds(R1, S - R1)]),
        (wqkv_hbm.at[:, pl.ds(2 * D, D)], wv_v),
        (wo_hbm, wo_v),
        (gw_hbm, gw_v),
        (wg_hbm, wg_v),
        (wu_hbm, wu_v),
        (wd_hbm, wd_v),
    ]
    cps = [pltpu.make_async_copy(s, d, sem.at[n]) for n, (s, d) in enumerate(pairs)]
    for c in cps:
        c.start()
    cp_wq, cp_x2, cp_wv, cp_wo, cp_gw, cp_wg, cp_wu, cp_wd = cps[n_stage:]

    def pair_gather(ref, base, n):
        return jnp.concatenate(
            [ref[pl.ds(base + p, n, stride=NP), :] for p in range(NP)], axis=0)

    def kp_accumulate(k, xt, first):
        pk = _phi(k)
        zz = jnp.sum(pk.reshape(pk.shape[0] // 8, 8, D), axis=0)
        pp = _dot(pk.astype(BF16).T, xt)
        if first:
            z_v[...] = zz
            p_v[...] = pp
        else:
            z_v[...] += zz
            p_v[...] += pp

    def q_matmul(row, rows):
        return lax.dot_general(x_v[pl.ds(row, rows), :], wqp_v[...], NT,
                               preferred_element_type=F32)

    def phase1():
        for n, (ca, cb) in enumerate(K_STAGES):
            cps[2 * n].wait()
            cps[2 * n + 1].wait()
            for a in range(0, R1, KT):
                k = _dot(x_v[a:a + KT, ca:cb], wk_v[ca:cb, :])
                if ca > 0:
                    k = k_v[a:a + KT, :] + k
                if cb < D:
                    k_v[a:a + KT, :] = k
                else:
                    kp_accumulate(k, x_v[a:a + KT, :], a == 0)

        cp_wq.wait()
        cp_x2.wait()
        cp_wv.wait()
        cp_wo.wait()
        wqt = pltpu.bitcast(wq_v[...].T, U32)
        for j in range(NB):
            wqt_v[j, 0:D // 2, :] = wqt[:, j * LANES:(j + 1) * LANES]
        for j in range(NB):
            for p in range(NP):
                wqp_v[p * 2 * H:(p + 1) * 2 * H, j * LANES:(j + 1) * LANES] = pltpu.bitcast(
                    wqt_v[j, pl.ds(p, H, stride=NP), :], BF16)
        for a in range(R1, S, KT):
            xt = x_v[a:a + KT, :]
            kp_accumulate(_dot(xt, wk_v[...]), xt, False)

        z = jnp.sum(z_v[...], axis=0, keepdims=True)
        zhi = z.astype(BF16).astype(F32)
        rid = lax.broadcasted_iota(jnp.int32, (LANES, D), 0)
        zz = jnp.where(rid == 0, zhi, jnp.where(rid == 1, z - zhi, 0.0)).astype(BF16)
        zt_v[0:D // 2, :] = pltpu.bitcast(zz.T, U32)
        zp = pltpu.bitcast(pair_gather(zt_v, 0, H), BF16).T.astype(F32)
        zp_v[...] = jnp.broadcast_to(zp[0:1, :] + zp[1:2, :], (8, D))

        q0_v[0:TS, :] = q_matmul(0, TS)
        same_head = (lax.broadcasted_iota(jnp.int32, (LANES, LANES), 0) // DH
                     == lax.broadcasted_iota(jnp.int32, (LANES, LANES), 1) // DH)
        for j in range(NB):
            sl = slice(j * LANES, (j + 1) * LANES)
            kv = _dot(p_v[sl, :].astype(BF16), wv_v[:, sl])
            kv_v[j * 64:(j + 1) * 64, :] = pltpu.bitcast(
                jnp.where(same_head, kv, 0.0).astype(BF16), U32)
        for it in range(1, n_iter):
            q0_v[it * TS:(it + 1) * TS, :] = q_matmul(it * T2, TS)
        for j in range(NB):
            kvp = pltpu.bitcast(pair_gather(kv_v, j * 64, HB), BF16)
            mj = _dot(kvp, wo_v[j * LANES:(j + 1) * LANES, :]).astype(BF16)
            for p in range(NP):
                dst = p * 2 * H + j * 2 * HB
                m_v[dst:dst + 2 * HB, :] = mj[p * 2 * HB:(p + 1) * 2 * HB, :]

        cp_gw.wait()
        cp_wg.wait()
        cp_wu.wait()
        cp_wd.wait()

    def write_out(row, rows, col, cols, val):
        o_v[pl.ds(row, rows), col:col + cols] = val
        pltpu.make_async_copy(o_v.at[pl.ds(row, rows), pl.ds(col, cols)],
                              o_hbm.at[pl.ds(row, rows), pl.ds(col, cols)], osem).start()

    def ffn_chunk(xt, c):
        hg = 0.5 * _dot(xt, wg_v[:, c:c + fc])
        up = _dot(xt, wu_v[:, c:c + fc])
        h = (hg * (jnp.tanh(hg) + 1.0)) * up
        return _dot(h.astype(BF16), wd_v[c:c + fc, :])

    def body(it, carry):
        pl.when(it == 0)(phase1)
        for si in range(n_sub):
            row = pl.multiple_of(it * T2 + si * TS, TS)
            xt = x_v[pl.ds(row, TS), :]
            gw = gw_v[...].astype(F32).reshape(1, D)
            g = _sigmoid(jnp.sum(xt.astype(F32) * gw, axis=1, keepdims=True))
            g = jnp.broadcast_to(g, (TS, LANES))

            b = ffn_chunk(xt, 0)

            if si == 0:
                q = q0_v[pl.ds(pl.multiple_of(it * TS, TS), TS), :]
            else:
                q = q_matmul(row, TS)
            pq = _phi(q)
            t = pq * zp_v[0:1, :]
            den = t[:, 0:LANES]
            for j in range(1, NB):
                den = den + t[:, j * LANES:(j + 1) * LANES]
            den = den + pltpu.roll(den, 2 * H, 1)
            even = lax.broadcasted_iota(jnp.int32, (TS, LANES), 1) % 2 == 0
            den = den + jnp.where(even, pltpu.roll(den, LANES - 1, 1), pltpu.roll(den, 1, 1))
            scale = g * pl.reciprocal(den + 1e-6, approx=False)
            r = jnp.concatenate(
                [(pq[:, j * LANES:(j + 1) * LANES] * scale).astype(BF16) for j in range(NB)],
                axis=1)

            b = b + ffn_chunk(xt, fc)
            b = b * jnp.concatenate([1.0 - g] * NB, axis=1)
            res = (_dot(r, m_v[...]) + b).astype(o_v.dtype)

            if si == n_sub - 1:
                half = D // 2
                write_out(row, TS, 0, half, res[:, 0:half])
                for a in range(0, TS, TAIL_ROWS):
                    write_out(pl.multiple_of(row + a, TAIL_ROWS), TAIL_ROWS, half, half,
                              res[a:a + TAIL_ROWS, half:D])
            else:
                write_out(row, TS, 0, D, res)
        return carry

    lax.fori_loop(0, n_iter, body, 0)
    pltpu.make_async_copy(o_v, o_hbm, osem).wait()


@jax.jit
def pallas_gated_mix__linear_attn_block__swiglu_ffn__prompt_kernel(
    A_x: jax.Array,
    A_wqkv: jax.Array,
    A_wo: jax.Array,
    B_x: jax.Array,
    B_w_gate: jax.Array,
    B_w_up: jax.Array,
    B_w_down: jax.Array,
    gate_w: jax.Array,
):
    del B_x
    B, S, D = A_x.shape
    F = B_w_gate.shape[1]
    assert B == 1 and S % T2 == 0 and (S - R1) % KT == 0 and S > R1
    assert D == 4 * LANES and F % (2 * LANES) == 0
    hbm = pl.BlockSpec(memory_space=pl.ANY)
    pad = D // 2 + 8
    no_checks = {name: True for name in ("disable_semaphore_checks", "disable_bounds_checks")
                 if hasattr(pltpu.CompilerParams, name)}
    out = pl.pallas_call(
        _kernel,
        out_shape=jax.ShapeDtypeStruct((S, D), A_x.dtype),
        in_specs=[hbm] * 7,
        out_specs=hbm,
        scratch_shapes=[
            pltpu.VMEM((S, D), BF16),
            pltpu.VMEM((D, D), BF16),
            pltpu.VMEM((D, D), BF16),
            pltpu.VMEM((D, D), BF16),
            pltpu.VMEM((D, D), BF16),
            pltpu.VMEM((D, F), BF16),
            pltpu.VMEM((D, F), BF16),
            pltpu.VMEM((F, D), BF16),
            pltpu.VMEM((D,), BF16),
            pltpu.VMEM((D, D), BF16),
            pltpu.VMEM((D // LANES, pad, LANES), U32),
            pltpu.VMEM((R1, D), F32),
            pltpu.VMEM((D, D), F32),
            pltpu.VMEM((8, D), F32),
            pltpu.VMEM((pad, LANES), U32),
            pltpu.VMEM((pad, LANES), U32),
            pltpu.VMEM((D, D), BF16),
            pltpu.VMEM((S // T2 * TS, D), F32),
            pltpu.VMEM((8, D), F32),
            pltpu.VMEM((S, D), A_x.dtype),
            pltpu.SemaphoreType.DMA((2 * len(K_STAGES) + 8,)),
            pltpu.SemaphoreType.DMA(()),
        ],
        compiler_params=pltpu.CompilerParams(vmem_limit_bytes=64 * 1024 * 1024, **no_checks),
    )(A_x.reshape(S, D), A_wqkv, A_wo, B_w_gate, B_w_up, B_w_down, gate_w)
    return out.reshape(B, S, D)
```

```python
import jax
import jax.numpy as jnp
from jax import lax
import jax.experimental.pallas as pl
import jax.experimental.pallas.tpu as pltpu

F32 = jnp.float32
BF16 = jnp.bfloat16
U32 = jnp.uint32
NT = (((1,), (1,)), ((), ()))

H = 32
LANES = 128
KT = 512
TS = 256
T2 = 1024
R1 = 1024
K_STAGES = ((0, 128), (128, 256), (256, 512))
Q_PRE = 3
KV_GROUP = 8
KV_LAG = 2
TAIL_ROWS = 32


def _phi(t):
    return jnp.where(t > 0, t + 1.0, jnp.exp(t)) + 1e-6


def _sigmoid(t):
    return 0.5 * jnp.tanh(0.5 * t) + 0.5


def _dot(a, b):
    return jnp.dot(a, b, preferred_element_type=F32)


def _kernel(x_hbm, wqkv_hbm, wo_hbm, wg_hbm, wu_hbm, wd_hbm, gw_hbm, o_hbm,
            x_v, wq_v, wk_v, wv_v, wo_v, wg_v, wu_v, wd_v, gw_v,
            wqp_v, wqt_v, wvt_v, k_v, p_v, z_v, zt_v, kv_v, m_v, q0_v, zp_v, o_v, sem, osem):
    S, D = x_v.shape
    F = wg_v.shape[1]
    DH = D // H
    NB = D // LANES
    NP = DH // 2
    HB = LANES // DH
    n_iter = S // T2
    n_sub = T2 // TS
    fc = F // 2

    pairs = []
    for ca, cb in K_STAGES:
        pairs.append((x_hbm.at[pl.ds(0, R1), pl.ds(ca, cb - ca)],
                      x_v.at[pl.ds(0, R1), pl.ds(ca, cb - ca)]))
        pairs.append((wqkv_hbm.at[pl.ds(ca, cb - ca), pl.ds(D, D)], wk_v.at[pl.ds(ca, cb - ca)]))
    n_stage = len(pairs)
    pairs += [
        (wqkv_hbm.at[:, pl.ds(0, D)], wq_v),
        (x_hbm.at[pl.ds(R1, S - R1)], x_v.at[pl.ds(R1, S - R1)]),
        (wqkv_hbm.at[:, pl.ds(2 * D, D)], wv_v),
        (wo_hbm, wo_v),
        (gw_hbm, gw_v),
        (wg_hbm, wg_v),
        (wu_hbm, wu_v),
        (wd_hbm, wd_v),
    ]
    cps = [pltpu.make_async_copy(s, d, sem.at[n]) for n, (s, d) in enumerate(pairs)]
    for c in cps:
        c.start()
    cp_wq, cp_x2, cp_wv, cp_wo, cp_gw, cp_wg, cp_wu, cp_wd = cps[n_stage:]

    def pair_gather(ref, base, n):
        return jnp.concatenate(
            [ref[pl.ds(base + p, n, stride=NP), :] for p in range(NP)], axis=0)

    def kp_accumulate(k, xt, first):
        pk = _phi(k)
        zz = jnp.sum(pk.reshape(pk.shape[0] // 8, 8, D), axis=0)
        pp = _dot(pk.astype(BF16).T, xt)
        if first:
            z_v[...] = zz
            p_v[...] = pp
        else:
            z_v[...] += zz
            p_v[...] += pp

    def q_matmul(row, rows):
        return lax.dot_general(x_v[pl.ds(row, rows), :], pltpu.bitcast(wqp_v[...], BF16), NT,
                               preferred_element_type=F32)

    def phase1():
        for n, (ca, cb) in enumerate(K_STAGES):
            cps[2 * n].wait()
            cps[2 * n + 1].wait()
            for a in range(0, R1, KT):
                k = _dot(x_v[a:a + KT, ca:cb], wk_v[ca:cb, :])
                if ca > 0:
                    k = k_v[a:a + KT, :] + k
                if cb < D:
                    k_v[a:a + KT, :] = k
                else:
                    kp_accumulate(k, x_v[a:a + KT, :], a == 0)

        cp_wq.wait()
        cp_x2.wait()
        cp_wv.wait()
        cp_wo.wait()
        wvt_v[...] = wv_v[...].T.astype(F32)
        wqt = pltpu.bitcast(wq_v[...].T, U32)
        for j in range(NB):
            wqt_v[j, 0:D // 2, :] = wqt[:, j * LANES:(j + 1) * LANES]
        wqp_v[...] = jnp.concatenate([pair_gather(wqt_v.at[j], 0, H) for j in range(NB)], axis=1)
        for a in range(R1, S, KT):
            xt = x_v[a:a + KT, :]
            kp_accumulate(_dot(xt, wk_v[...]), xt, False)

        z = jnp.sum(z_v[...], axis=0, keepdims=True)
        zhi = z.astype(BF16).astype(F32)
        rid = lax.broadcasted_iota(jnp.int32, (LANES, D), 0)
        zz = jnp.where(rid == 0, zhi, jnp.where(rid == 1, z - zhi, 0.0)).astype(BF16)
        zt_v[0:D // 2, :] = pltpu.bitcast(zz.T, U32)
        zp = pltpu.bitcast(pair_gather(zt_v, 0, H), BF16).T.astype(F32)
        zp_v[...] = jnp.broadcast_to(zp[0:1, :] + zp[1:2, :], (8, D))

        lane = lax.broadcasted_iota(jnp.int32, (DH, LANES), 1)
        done = []
        for h in range(H):
            p_h = p_v[h * DH:(h + 1) * DH, :]
            blk = jnp.zeros((DH, LANES), F32)
            for e in range(DH):
                if e % KV_GROUP == 0:
                    ph = p_h
                    if len(done) >= KV_LAG:
                        zero = jnp.minimum(jnp.abs(done[-KV_LAG]), 0.0)
                        ph = p_h + jnp.concatenate([zero] * NB, axis=1)
                col = jnp.sum(ph * wvt_v[h * DH + e:h * DH + e + 1, :], axis=1, keepdims=True)
                blk = jnp.where(lane == (h % HB) * DH + e, col, blk)
                if e % KV_GROUP == KV_GROUP - 1:
                    done.append(blk)
            kv_v[h * NP:(h + 1) * NP, :] = pltpu.bitcast(blk.astype(BF16), U32)
        for it in range(n_iter):
            for si in range(Q_PRE):
                n = it * Q_PRE + si
                q0_v[n * TS:(n + 1) * TS, :] = q_matmul(it * T2 + si * TS, TS)
        for j in range(NB):
            kvp = pltpu.bitcast(pair_gather(kv_v, j * 64, HB), BF16)
            mj = _dot(kvp, wo_v[j * LANES:(j + 1) * LANES, :]).astype(BF16)
            for p in range(NP):
                dst = p * 2 * H + j * 2 * HB
                m_v[dst:dst + 2 * HB, :] = mj[p * 2 * HB:(p + 1) * 2 * HB, :]

        cp_gw.wait()
        cp_wg.wait()
        cp_wu.wait()
        cp_wd.wait()

    def write_out(row, rows, col, cols, val):
        o_v[pl.ds(row, rows), col:col + cols] = val
        pltpu.make_async_copy(o_v.at[pl.ds(row, rows), pl.ds(col, cols)],
                              o_hbm.at[pl.ds(row, rows), pl.ds(col, cols)], osem).start()

    def ffn_chunk(xt, c):
        hg = 0.5 * _dot(xt, wg_v[:, c:c + fc])
        up = _dot(xt, wu_v[:, c:c + fc])
        h = (hg * (jnp.tanh(hg) + 1.0)) * up
        return _dot(h.astype(BF16), wd_v[c:c + fc, :])

    def body(it, carry):
        pl.when(it == 0)(phase1)
        for si in range(n_sub):
            row = pl.multiple_of(it * T2 + si * TS, TS)
            xt = x_v[pl.ds(row, TS), :]
            gw = gw_v[...].astype(F32).reshape(1, D)
            g = _sigmoid(jnp.sum(xt.astype(F32) * gw, axis=1, keepdims=True))
            g = jnp.broadcast_to(g, (TS, LANES))

            b = ffn_chunk(xt, 0)

            if si < Q_PRE:
                q = q0_v[pl.ds(pl.multiple_of((it * Q_PRE + si) * TS, TS), TS), :]
            else:
                q = q_matmul(row, TS)
            pq = _phi(q)
            t = pq * zp_v[0:1, :]
            den = t[:, 0:LANES]
            for j in range(1, NB):
                den = den + t[:, j * LANES:(j + 1) * LANES]
            den = den + pltpu.roll(den, 2 * H, 1)
            even = lax.broadcasted_iota(jnp.int32, (TS, LANES), 1) % 2 == 0
            den = den + jnp.where(even, pltpu.roll(den, LANES - 1, 1), pltpu.roll(den, 1, 1))
            scale = g * pl.reciprocal(den + 1e-6, approx=False)
            r = (pq * jnp.concatenate([scale] * NB, axis=1)).astype(BF16)

            b = b + ffn_chunk(xt, fc)
            b = b * jnp.concatenate([1.0 - g] * NB, axis=1)
            res = (_dot(r, m_v[...]) + b).astype(o_v.dtype)

            if si == n_sub - 1:
                half = D // 2
                write_out(row, TS, 0, half, res[:, 0:half])
                for a in range(0, TS, TAIL_ROWS):
                    write_out(pl.multiple_of(row + a, TAIL_ROWS), TAIL_ROWS, half, half,
                              res[a:a + TAIL_ROWS, half:D])
            else:
                write_out(row, TS, 0, D, res)
        return carry

    lax.fori_loop(0, n_iter, body, 0)
    pltpu.make_async_copy(o_v, o_hbm, osem).wait()


@jax.jit
def pallas_gated_mix__linear_attn_block__swiglu_ffn__prompt_kernel(
    A_x: jax.Array,
    A_wqkv: jax.Array,
    A_wo: jax.Array,
    B_x: jax.Array,
    B_w_gate: jax.Array,
    B_w_up: jax.Array,
    B_w_down: jax.Array,
    gate_w: jax.Array,
):
    del B_x
    B, S, D = A_x.shape
    F = B_w_gate.shape[1]
    assert B == 1 and S % T2 == 0 and (S - R1) % KT == 0 and S > R1
    assert D == 4 * LANES and F % (2 * LANES) == 0
    hbm = pl.BlockSpec(memory_space=pl.ANY)
    pad = D // 2 + 8
    no_checks = {name: True for name in ("disable_semaphore_checks", "disable_bounds_checks")
                 if hasattr(pltpu.CompilerParams, name)}
    out = pl.pallas_call(
        _kernel,
        out_shape=jax.ShapeDtypeStruct((S, D), A_x.dtype),
        in_specs=[hbm] * 7,
        out_specs=hbm,
        scratch_shapes=[
            pltpu.VMEM((S, D), BF16),
            pltpu.VMEM((D, D), BF16),
            pltpu.VMEM((D, D), BF16),
            pltpu.VMEM((D, D), BF16),
            pltpu.VMEM((D, D), BF16),
            pltpu.VMEM((D, F), BF16),
            pltpu.VMEM((D, F), BF16),
            pltpu.VMEM((F, D), BF16),
            pltpu.VMEM((D,), BF16),
            pltpu.VMEM((D // 2, D), U32),
            pltpu.VMEM((D // LANES, pad, LANES), U32),
            pltpu.VMEM((D, D), F32),
            pltpu.VMEM((R1, D), F32),
            pltpu.VMEM((D, D), F32),
            pltpu.VMEM((8, D), F32),
            pltpu.VMEM((pad, LANES), U32),
            pltpu.VMEM((pad, LANES), U32),
            pltpu.VMEM((D, D), BF16),
            pltpu.VMEM((S // T2 * Q_PRE * TS, D), F32),
            pltpu.VMEM((8, D), F32),
            pltpu.VMEM((S, D), A_x.dtype),
            pltpu.SemaphoreType.DMA((2 * len(K_STAGES) + 8,)),
            pltpu.SemaphoreType.DMA(()),
        ],
        compiler_params=pltpu.CompilerParams(vmem_limit_bytes=64 * 1024 * 1024, **no_checks),
    )(A_x.reshape(S, D), A_wqkv, A_wo, B_w_gate, B_w_up, B_w_down, gate_w)
    return out.reshape(B, S, D)
```
